```python
import jax
import jax.numpy as jnp

def _softmax(x, axis=-1):
    return jax.nn.softmax(x, axis=axis)
def _gelu(x):
    return jax.nn.gelu(x, approximate=True)
def _silu(x):
    return jax.nn.silu(x)
def _sigmoid(x):
    return jax.nn.sigmoid(x)
def _layernorm(x, axis=-1, eps=1e-5):
    m = jnp.mean(x, axis=axis, keepdims=True)
    v = jnp.var(x, axis=axis, keepdims=True)
    return (x - m) / jnp.sqrt(v + eps)
def _scatter_add(tgt, idx, src, axis=0):
    return tgt.at[idx].add(src)
def _segment_sum(src, seg, n):
    return jax.ops.segment_sum(src, seg, n)
class _Rng:
    def __init__(self, key):
        self._k = key
    def _next(self):
        self._k, sub = jax.random.split(self._k)
        return sub
    def normal(self, shape):
        return jax.random.normal(self._next(), shape, dtype=jnp.bfloat16)
    def randint(self, lo, hi, shape):
        return jax.random.randint(self._next(), shape, lo, hi, dtype=jnp.int32)
    def uniform(self, shape, lo=0.0, hi=1.0):
        return jax.random.uniform(self._next(), shape, jnp.bfloat16, lo, hi)
    def permutation(self, n):
        return jax.random.permutation(self._next(), n)


kernel_name = 'standalone__modern_conv_block_slak__vision'

def setup_inputs():
    _rng = _Rng(jax.random.key(int.from_bytes(__import__("os").urandom(4), "little")))
    _w = (lambda a: (lambda t: t.astype(jnp.bfloat16) if jnp.issubdtype(t.dtype, jnp.floating) else t)(jnp.asarray(a)))
    H = W = 384
    C = 384
    K = 1
    return {
        "x": _w((lambda *s: _rng.normal(s) * 0.05)(1, H, W, C)),
        "dw": _w((lambda *s: _rng.normal(s) * 0.05)(K, K, C)),
        "w1": _w((lambda *s: _rng.normal(s) * 0.05)(C, 4 * C)),
        "w2": _w((lambda *s: _rng.normal(s) * 0.05)(4 * C, C)),
        "grn_g": _w((lambda *s: _rng.normal(s) * 0.05)(4 * C)),
        "grn_b": _w((lambda *s: _rng.normal(s) * 0.05)(4 * C)),
    }

def reference(x, dw, w1, w2, grn_g, grn_b):
    B, H, W, C = x.shape
    K = dw.shape[0]
    pad = K // 2
    xp = jnp.pad(x, ((0,0),(pad,pad),(pad,pad),(0,0)))
    out = jnp.zeros_like(x)
    for i in range(K):
        for j in range(K):
            out = out + xp[:, i:i+H, j:j+W, :] * dw[i, j][None, None, None, :]
    h = _layernorm(out, axis=-1)
    h = _gelu(h @ w1)
    gx = jnp.sqrt((h * h).sum(axis=(1, 2), keepdims=True) + 1e-6)
    nx = gx / (gx.mean(axis=-1, keepdims=True) + 1e-6)
    h = grn_g[None, None, None, :] * (h * nx) + grn_b[None, None, None, :] + h
    return x + h @ w2
```

```python
import jax
import jax.numpy as jnp
import numpy as np
from jax import lax
import jax.experimental.pallas as pl
import jax.experimental.pallas.tpu as pltpu

_C0 = float(np.sqrt(2.0 / np.pi))
_C1 = _C0 * 0.044715
_A = _C1 ** (1.0 / 3.0)
_K0 = _C0 / _A
_GS = 0.5 / _A


def lincomb(terms, get):
    pos = [v for v, c in terms if c > 0]
    neg = [v for v, c in terms if c < 0]
    sign = 1
    if not pos:
        pos, neg, sign = neg, [], -1
    acc = get(pos[0])
    for v, c in terms:
        if v == pos[0]:
            continue
        acc = acc + get(v) if c * sign > 0 else acc - get(v)
    return acc, sign


class Lazy:
    def __init__(self, nin, steps, leaf):
        self.nin, self.steps, self.leaf, self.memo = nin, steps, leaf, {}
    def __call__(self, v):
        if v not in self.memo:
            if v < self.nin:
                self.memo[v] = self.leaf(v)
            else:
                i, j, s = self.steps[v - self.nin]
                self.memo[v] = self(i) + self(j) if s > 0 else self(i) - self(j)
        return self.memo[v]


def cse(rows):
    R = [list(map(int, r)) for r in rows]; steps = []
    while True:
        n = len(R[0]); best = 1; arg = None
        for i in range(n):
            for j in range(i+1, n):
                a = sum(1 for r in R if r[i]*r[j] > 0); b = sum(1 for r in R if r[i]*r[j] < 0)
                if a > best: best = a; arg = (i, j, 1)
                if b > best: best = b; arg = (i, j, -1)
        if arg is None: break
        i, j, s = arg; steps.append(arg)
        for r in R:
            if r[i]*r[j] == s: r.append(r[i]); r[i] = 0; r[j] = 0
            else: r.append(0)
    return steps, [[(v, c) for v, c in enumerate(r) if c] for r in R]

SCHEMES = {
    'fg/p233_2.txt': ((2, 3, 3), [[0, 0, 0, 0, 0, 1], [1, 0, 0, -1, 1, 0], [0, -1, -1, 0, 0, 1], [1, 0, 1, 0, 0, 0], [0, 0, 0, -1, 0, -1], [-1, 0, 0, 0, 0, -1], [0, 1, 0, 0, 0, 0], [0, 0, 1, 0, 0, -1], [-1, 0, 0, 0, 0, 0], [0, -1, -1, 0, 1, 1], [0, 0, 0, 0, 1, 0], [-1, 1, 0, 1, -1, 0], [0, 0, 0, 1, -1, 0], [0, -1, -1, 0, 0, 0], [1, 0, 0, -1, 0, 0]], [[1, 0, 1, 0, 0, 0, -1, 0, 0], [0, 0, -1, 0, -1, 0, 0, 0, 0], [0, 0, 0, -1, 0, -1, 0, 0, 1], [0, 0, 0, 0, 0, 0, 0, -1, 0], [-1, 0, -1, 0, 0, 0, 0, 0, 0], [1, 0, 1, 0, 0, 0, 0, -1, 0], [0, 0, 0, 0, -1, 1, 0, 0, -1], [0, 0, 0, -1, 0, -1, 1, -1, 1], [0, 1, -1, 0, 0, 0, 0, -1, 0], [0, 0, 0, 1, 0, 1, 0, 0, 0], [0, 0, -1, 1, 0, 0, 0, 0, 0], [0, 0, 0, 0, 1, 0, 0, 0, 0], [0, 0, 1, 0, 0, 0, 0, 0, 0], [0, 0, 0, 0, 0, 0, 0, 0, -1], [-1, 1, -1, 0, 1, 0, 0, 0, 0]], [[-1, 0, 0, -1, 0, 0], [1, -1, -1, 0, -1, 0], [1, 0, 0, 0, 0, 1], [-1, -1, 0, 0, 0, 0], [0, 0, 0, 1, 1, 0], [-1, 0, 0, 0, 1, 0], [-1, 0, 1, 0, 0, 0], [1, 0, 0, 0, 0, 0], [0, -1, 0, 0, -1, 0], [0, 0, 0, 0, 0, 1], [0, 0, 0, 1, 0, -1], [-1, 1, 1, 0, 0, 0], [-1, 1, 1, -1, 1, 1], [0, 0, 1, 0, 0, 1], [0, 0, 0, 0, -1, 0]]),
    'fg/p233_4.txt': ((2, 3, 3), [[0, 0, 0, 0, 0, -1], [-1, -1, 0, -1, -1, 0], [1, 0, 1, 0, 0, 0], [1, 0, 0, 0, 0, 0], [0, 0, 0, 0, 1, 0], [-1, -1, 0, 0, 0, -1], [1, 1, 0, 0, 1, 0], [0, 0, 0, -1, 0, 0], [0, 0, -1, 0, 0, -1], [0, 1, 0, 0, 1, 0], [-1, 0, -1, 0, 0, -1], [-1, -1, 1, 0, 0, 0], [-1, 0, -1, -1, 0, -1], [0, 0, 0, 1, 1, -1], [-1, -1, 0, 0, 0, 0]], [[0, 0, 0, -1, 0, 0, -1, 1, 0], [0, 0, 1, 1, 0, 0, 0, 0, 0], [0, 0, 0, 0, 0, 0, 0, -1, 0], [0, 1, -1, 0, -1, 1, 0, -1, 0], [0, 0, 0, 0, -1, 0, 0, 0, 0], [0, 0, 0, -1, 0, 0, 0, 0, 1], [0, 0, -1, 0, -1, 1, 0, 0, 0], [-1, 1, 0, 1, 0, 0, 0, 0, 0], [-1, 0, 0, 1, 0, 0, 1, 0, 1], [0, 0, 1, 0, 0, -1, 0, 0, 0], [1, 0, 0, -1, 0, 0, 0, -1, 0], [0, 0, 0, 0, 0, 0, 0, 0, -1], [-1, 0, 0, 1, 0, 0, 0, 0, 0], [0, 0, 0, 1, 0, 0, 0, 0, 0], [0, 0, 0, 0, -1, 1, 0, 0, 1]], [[-1, 0, 0, 1, 0, 0], [0, 0, 0, 0, 0, -1], [-1, -1, 0, 1, 1, 0], [0, 1, 0, 0, 0, 0], [0, 1, 1, 0, -1, -1], [1, 0, 0, 0, 0, -1], [0, -1, -1, 0, 0, 1], [0, 0, 0, 0, -1, 0], [-1, 0, 0, 0, 0, 0], [0, -1, -1, 0, 0, 0], [-1, 0, 0, 1, 1, 0], [1, 0, -1, 0, 0, 0], [0, 0, 0, 1, 1, 0], [0, 0, 0, 1, 0, -1], [0, 0, -1, 0, 0, 1]]),
}


def load_scheme(name):
    sh, U, V, W = SCHEMES[name]
    return sh, np.array(U), np.array(V), np.array(W)


L = 128
u32 = jnp.uint32


def schedule(T, S, NS, D):
    spread = S - NS
    keep = [((i + 1) * spread) // (T - NS) > (i * spread) // (T - NS) for i in range(T - NS)] + [True] * NS
    slot1, spill, wait1, last, nxt, rr, nsp = [], [], [], {}, NS, 0, 0
    for i in range(T):
        if keep[i] and i < T - NS:
            slot1.append(nxt); wait1.append(-1); nxt += 1
        else:
            slot1.append(rr); wait1.append(last.get(rr, -1)); last[rr] = i; rr = (rr + 1) % NS
        spill.append(-1 if keep[i] else nsp)
        nsp += not keep[i]
    kept = [i for i in range(T) if keep[i]][::-1]
    rest = [i for i in range(T) if not keep[i]]
    order, nk = kept[:D], len(kept) - D
    kept = kept[D:]
    for j in range(T - D):
        order.append(kept.pop(0) if ((j + 1) * nk) // (T - D) > (j * nk) // (T - D) else rest.pop(0))
    slot2 = []
    for j, i in enumerate(order):
        slot2.append(slot1[i] if keep[i] else slot2[j - D])
    src2 = [spill[i] for i in order]
    wsp = [spill[w] if w >= 0 else -1 for w in wait1]
    return np.array([slot1, spill, wsp, order, slot2, src2], np.int32), nsp


def build(RB1=256, U1=2, RB2=256, U2=2, NX=4, NO=3, px=0, delay=0, xfirst=False, po=0, ph=0, S=30, NS=4, D=5, vmem_mb=128, phase=3, dma=True, s1='fg/p233_4.txt', s2='fg/p233_2.txt',
          MT1=8, MT2=16, LT=16, flags=None, lag1=12, lag2=1, lnlo=0.0, lnhi=0.9, cblo=0.0, cbhi=0.9, order1=None, order2=None,
          wide1=1, split2=False, lsync=False, NM=4, ST=16, ST2=32, MS=4, hsync=True, xs2=True, gsync=1, pj=-1, LN=8, lnlag=12, nln=4, bsync=-1, gd=5, gmode=0, dsrc=0, async_=True, pdel=2, asy=-1, pmode=8, mdel=4, zm=1, zl=1, za=1):
    def fn(x, dw, w1, w2, grn_g, grn_b):
        B, H, W, C = x.shape
        F = w1.shape[1]
        N = B * H * W
        f32, bf16 = jnp.float32, jnp.bfloat16
        (m1, k1, n1), Us1, Vs1, Ws1 = load_scheme(s1)
        (m2, k2, n2), Us2, Vs2, Ws2 = load_scheme(s2)
        if order1 is not None: Us1, Vs1, Ws1 = Us1[order1], Vs1[order1], Ws1[order1]
        if order2 is not None: Us2, Vs2, Ws2 = Us2[order2], Vs2[order2], Ws2[order2]
        R1, R2 = len(Us1), len(Us2)
        assert k1 * L == C and n2 * L == C
        G1 = F // (n1 * L)
        G2 = F // (k2 * L)
        a1_steps, a1_out = cse(Us1)
        c1_steps, c1_out = cse(Ws1.T)
        a2_steps, a2_out = cse(Us2)
        c2_steps, c2_out = cse(Ws2.T)
        sg1 = [1 if any(c > 0 for _, c in t) else -1 for t in a1_out]
        sg2 = [1 if any(c > 0 for _, c in t) else -1 for t in a2_out]
        CM1, CM2 = m1 * RB1, m2 * RB2
        TM = CM1 * U1
        assert TM == CM2 * U2 and N % TM == 0
        T = N // TM
        NT = F // L
        direct2 = [len(t) == 1 and t[0][0] < m2 * k2 for t in a2_out]
        assert (U1 * G1) % MS == 0
        GA = G1 // wide1

        tab, nsp = schedule(T, S, NS, D)
        HS = NT * TM

        def kernel(tab_ref, x_hbm, dw_ref, w1_ref, w2_ref, g_ref, b_ref, o_hbm, h_hbm,
                   xbuf, hbuf, obuf, b1, b2, acc, bias, zero, dwf, lnbuf, a1e, a1o, a2buf, m2buf, xsem, hsem, osem, *mbs):
            a1b = (a1e, a1o)
            class _Nop:
                def start(self, priority=0): pass
                def wait(self): pass
            mk = pltpu.make_async_copy if dma else (lambda *a: _Nop())
            def x_copy(i, s): return mk(x_hbm.at[pl.ds(i * TM, TM)], xbuf.at[s, pl.ds(0, TM)], xsem.at[s])
            def hw_copy(i, s): return mk(hbuf.at[s, pl.ds(0, HS)], h_hbm.at[i], hsem.at[s])
            def hr_copy(i, s): return mk(h_hbm.at[i], hbuf.at[s, pl.ds(0, HS)], hsem.at[s])
            def o_copy(i, s): return mk(obuf.at[s], o_hbm.at[pl.ds(i * TM, TM)], osem.at[s])
            def hrows(s, ct, row, n): return (s, pl.ds(ct * TM + row, n))
            def xrows(s, row, n): return (s, pl.ds(row, n))

            for j in range(NX):
                x_copy(j, j).start(priority=px)
            zero[0] = 0
            for ab in a1b:
                ab[R1 * RB1 // 2:R1 * RB1 // 2 + 16, :] = jnp.zeros((16, L), u32)
            acc[...] = jnp.zeros_like(acc)
            for mb in mbs:
                mb[...] = jnp.zeros_like(mb)
            dwf[...] = jnp.broadcast_to(dw_ref[...].astype(f32), dwf.shape)
            for g in range(G1):
                for r in range(R1):
                    def get(v):
                        ct = (v % n1) * G1 + g
                        return w1_ref[(v // n1) * L:(v // n1 + 1) * L, ct * L:(ct + 1) * L].astype(f32)
                    val, sg = lincomb([(v, int(c) * sg1[r]) for v, c in enumerate(Vs1[r]) if c], get)
                    b1[g * R1 + r] = pltpu.bitcast((val if sg > 0 else -val).astype(bf16), u32)

            def ln_rows(s, row):
                o = xbuf[xrows(s, row, LN)].astype(f32) * dwf[...]
                mu = jnp.sum(o, axis=-1, keepdims=True) * (1.0 / C)
                d = o - mu
                v = jnp.sum(d * d, axis=-1, keepdims=True) * (1.0 / C)
                return d * (lax.rsqrt(v + 1e-5) * _A)

            def a_combos(geta):
                av = Lazy(m1 * k1, a1_steps, geta)
                return [lincomb(a1_out[r], av)[0] for r in range(R1)]

            def ln_store(s, row, lrow):
                a = ln_rows(s, row)
                for j in range(k1):
                    lnbuf[j, pl.ds(lrow, LN), :] = a[:, j * L:(j + 1) * L]

            def ac_tile(lrow, dst, drow):
                ev, od = (a_combos(lambda v: lnbuf[v % k1, pl.ds(lrow + (v // k1) * LT + par, LT // 2, stride=2), :]) for par in range(2))
                for r in range(R1):
                    dst[pl.ds(drow + r * (RB1 // 2), LT // 2), :] = pltpu.pack_elementwise([ev[r], od[r]], packed_dtype=bf16)

            def gelu_rows(getm, g, sq):
                mv = Lazy(R1, c1_steps, getm)
                res = []
                for e in range(m1 * n1):
                    y, sg = lincomb(c1_out[e], mv)
                    th = jnp.tanh(y * (y * y + _K0))
                    hv = y * (th + 1.0) if sg > 0 else y * (th - 1.0)
                    ct = (e % n1) * G1 + g
                    p = hv * hv
                    for z in range(p.shape[0] // 8):
                        sq[ct] = sq[ct] + p[z * 8:(z + 1) * 8] if ct in sq else p[z * 8:(z + 1) * 8]
                    res.append(hv)
                return res

            def h_store(res, s, row0, g):
                for e, hv in enumerate(res):
                    hbuf[hrows(s, (e % n1) * G1 + g, row0 + (e // n1) * RB1, hv.shape[0])] = hv.astype(bf16)

            def gelu_tile(getm, s, row0, g, sq):
                h_store(gelu_rows(getm, g, sq), s, row0, g)

            def flush_sq(sq):
                for ct in sorted(sq):
                    acc[ct] += sq[ct]
                sq.clear()

            ND = U1 * G1 * R1
            assert ND % NM == 0
            tpr = RB1 // ST
            ntick = ND // NM * tpr
            nt = RB1 // MT1
            ge_at = [[] for _ in range(ntick)]
            for a in range(U1 * G1):
                ready = (((a + 1) * R1 - 1) // NM + 1) * tpr
                for t in range(nt):
                    z = max(((a + 1) * R1 * tpr) // NM + lag1 + (t * R1 * tpr) // (NM * nt),
                            ready)
                    if t % max(1, 16 // MT1) and z >= ntick > zprev:
                        z = ntick - 1
                    zprev = z
                    ge_at[z % ntick].append((a, t, z >= ntick))
            carried = sorted({(a, t) for ev in ge_at for a, t, c in ev if c})
            nl = RB1 // LT
            npq = LT // LN
            ln_at = [[] for _ in range(ntick)]
            ac_at = [[] for _ in range(ntick)]
            for u in range(U1):
                n_it = nl * m1 * npq
                for it in range(n_it):
                    z = int((u + lnlo + (lnhi - lnlo) * it / n_it) * ntick / U1)
                    ln_at[z].append((u + 1, it // (m1 * npq), (it // npq) % m1, it % npq))
                    if (it + 1) % (m1 * npq) == 0:
                        ac_at[z + lnlag].append((u + 1, it // (m1 * npq)))
            hp = max(1, 16 // MT1)

            def p1_body(s_prev, s_cur, sx_cur, sx_next, wr, rd, pin):
                parts = {}
                lhs = {}
                sq = {}
                held = []
                z0 = pl.multiple_of(zero[0], 8)
                done = []
                probes = []
                for rho in range(ND // NM):
                    res = []
                    for z in range(rho * NM, (rho + 1) * NM):
                        a, r = divmod(z, R1)
                        u, g = divmod(a, G1)
                        lhs = pltpu.bitcast(a1b[u % 2][r * (RB1 // 2):(r + 1) * (RB1 // 2), :], bf16)
                        res.append((a, r, jnp.dot(lhs, pltpu.bitcast(b1[g * R1 + r], bf16), preferred_element_type=f32)))
                    for k in range(tpr):
                        pv = res[pj][2][k * ST:k * ST + 8]
                        for a, r, val in res:
                            mbs[a % MS][pl.ds((z0 if zm else 0) + r * RB1 + k * ST, ST), :] = val[k * ST:(k + 1) * ST]
                        if pmode and k % pmode == pmode - 1:
                            for a2 in sorted({a3 for a3, _, _ in res}):
                                probes.append((len(done) + mdel, mbs[a2 % MS][R1 * RB1 + 16:R1 * RB1 + 24, :]))
                            probes.sort(key=lambda e: e[0])
                        if k == bsync:
                            b1[wr, 0:8, :] = pltpu.bitcast(pv, u32)
                        if k == asy:
                            a1b[((rho + 1) * NM // (R1 * G1)) % 2][pl.ds(rd - R1 * RB1 // 2, 8), :] = pltpu.bitcast(pv, u32)
                        for (pa, t, c) in ge_at[rho * tpr + k]:
                            pu, pg = divmod(pa, G1)
                            if t % gsync == 0:
                                if len(done) < gd:
                                    mbs[pa % MS][pl.ds(rd, 8), :] = pv
                                elif gmode == 0:
                                    val = done[-gd]
                                    val = val + pv
                                    while probes and probes[0][0] <= len(done):
                                        val = val + probes.pop(0)[1]
                                    mbs[pa % MS][pl.ds(rd, 8), :] = val
                                else:
                                    mbs[pa % MS][pl.ds(rd, 8), :] = done[-gd]
                            held.append(gelu_rows(lambda v: mbs[pa % MS][v * RB1 + t * MT1:v * RB1 + (t + 1) * MT1, :], pg, sq))
                            done.append(sum([sq[l * G1 + pg] for l in range(1, n1)], sq[pg]))
                            if len(held) == hp:
                                h_store([jnp.concatenate(hs, axis=0) for hs in zip(*held)], s_prev if c else s_cur,
                                        pu * CM1 + (t + 1 - hp) * MT1, pg)
                                held = []
                            if t == nt - 1:
                                flush_sq(sq)
                        for (nu, t, q, j) in ln_at[rho * tpr + k]:
                            if lsync:
                                xbuf[pin, TM:TM + 8, 0:L] = pv.astype(bf16)
                            ln_store(sx_cur if nu < U1 else sx_next, (nu % U1) * CM1 + q * RB1 + t * LT + j * LN,
                                     (z0 if zl else 0) + ((t % nln) * m1 + q) * LT + j * LN)
                        for (nu, t) in ac_at[rho * tpr + k]:
                            lnbuf[0, pl.ds(rd - R1 * RB1 + nln * m1 * LT, 8), :] = pv
                            ac_tile((t % nln) * m1 * LT, a1b[nu % 2], (z0 if za else 0) + t * (LT // 2))
                            if async_:
                                probes.append((len(done) + pdel, pltpu.bitcast(a1b[nu % 2][R1 * RB1 // 2:R1 * RB1 // 2 + 8, :], f32)))
                flush_sq(sq)

            if phase & 1:
                x_copy(0, 0).wait()
                def pro(t, _):
                    r0 = pl.multiple_of(t * LT, LT)
                    for q in range(m1):
                        for j in range(npq):
                            ln_store(0, r0 + q * RB1 + j * LN, q * LT + j * LN)
                    ac_tile(0, a1e, pl.multiple_of(t * (LT // 2), LT // 2))
                lax.fori_loop(0, RB1 // LT, pro, None)

                def p1(i, _):
                    ip = jnp.maximum(i - 1, 0)

                    @pl.when(i + 1 < T)
                    def _():
                        x_copy(i + 1, lax.rem(i + 1, NX)).wait()

                    @pl.when(tab_ref[2, i] >= 0)
                    def _():
                        hw_copy(tab_ref[2, i], tab_ref[0, i]).wait()
                    par = lax.rem(i, 2)
                    p1_body(jnp.where(i > 0, tab_ref[0, ip], S - 1), tab_ref[0, i], lax.rem(i, NX), lax.rem(jnp.minimum(i + 1, T - 1), NX),
                            G1 * R1 + par, pl.multiple_of(R1 * RB1 + 8 * par, 8), par)

                    @pl.when(i + NX < T)
                    def _():
                        x_copy(i + NX, lax.rem(i, NX)).start(priority=px)

                    @pl.when(jnp.logical_and(i >= 1, tab_ref[1, ip] >= 0))
                    def _():
                        hw_copy(tab_ref[1, ip], tab_ref[0, ip]).start(priority=ph)
                lax.fori_loop(0, T, p1, None)
                if phase & 2:
                    for j in range(NX - 1):
                        x_copy(int(tab[3, j]), j).start(priority=px)

                for a in sorted({a for a, _ in carried}):
                    def epi(t, _):
                        sq = {}
                        r0 = pl.multiple_of(t * MT1, MT1)
                        gelu_tile(lambda v: mbs[a % MS][pl.ds(v * RB1 + r0, MT1), :], int(tab[0, T - 1]), (a // G1) * CM1 + r0, a % G1, sq)
                        flush_sq(sq)
                    lax.fori_loop(min(t for ca, t in carried if ca == a), nt, epi, None)
            else:
                for j in range(NX):
                    x_copy(j, j).wait()
                for j in range(NX - 1):
                    x_copy(j, j).start(priority=px)
            if not (phase & 2):
                return

            ss = jnp.concatenate([jnp.sum(acc[c], axis=0, keepdims=True) for c in range(NT)], axis=1) * (_GS * _GS)
            gx = jnp.sqrt(ss + 1e-6)
            nx = gx / (jnp.sum(gx, axis=-1, keepdims=True) * (1.0 / F) + 1e-6)
            sc = (g_ref[...].astype(f32) * nx + 1.0) * _GS
            sct = jnp.transpose(jnp.broadcast_to(sc, (L, F)))
            for q in range(G2):
                for r in range(R2):
                    def get(v):
                        ct = (v // n2) * G2 + q
                        return w2_ref[ct * L:(ct + 1) * L, (v % n2) * L:(v % n2 + 1) * L].astype(f32) * sct[ct * L:(ct + 1) * L]
                    val, sg = lincomb([(v, int(c) * sg2[r]) for v, c in enumerate(Vs2[r]) if c], get)
                    b2[r, q * L // 2:(q + 1) * L // 2, :] = pltpu.bitcast((val if sg > 0 else -val).astype(bf16), u32)
            bias[...] = jnp.dot(jnp.broadcast_to(b_ref[...], (8, F)), w2_ref[...], preferred_element_type=f32)
            m2buf[...] = jnp.zeros_like(m2buf)

            def comb_tile(s, row0, q):
                raw = Lazy(m2 * k2, [], lambda v: hbuf[hrows(s, (v % k2) * G2 + q, row0 + (v // k2) * RB2, MT2)])
                av = Lazy(m2 * k2, a2_steps, lambda v: raw(v).astype(f32))
                return [raw(a2_out[r][0][0]) if direct2[r] else lincomb(a2_out[r], av)[0].astype(bf16) for r in range(R2)]

            def out_tile(getm, sx, so, row0):
                mv = Lazy(R2, c2_steps, getm)
                for i in range(m2):
                    rows = pl.ds(row0 + i * RB2, MT2)
                    xv = xbuf[xrows(sx, row0 + i * RB2, MT2)].astype(f32)
                    res = []
                    for l in range(n2):
                        y, sg = lincomb(c2_out[i * n2 + l], mv)
                        z = xv[:, l * L:(l + 1) * L] + jnp.concatenate([bias[:, l * L:(l + 1) * L]] * (MT2 // 8), axis=0)
                        res.append(z + y if sg > 0 else z - y)
                    obuf[so, rows, :] = jnp.concatenate(res, axis=1).astype(bf16)

            tp2 = RB2 // ST2
            ntick2 = U2 * R2 * tp2
            nt2 = RB2 // MT2
            ot_at = [[] for _ in range(ntick2)]
            cb_at = [[] for _ in range(ntick2)]
            for u in range(U2):
                for t in range(nt2):
                    z = (u + 1) * R2 * tp2 + lag2 + (t * (R2 * tp2 - lag2)) // nt2
                    ot_at[z % ntick2].append((u, t, z >= ntick2))
                for k in range(G2 * nt2):
                    cb_at[int((u + cblo + (cbhi - cblo) * k / (G2 * nt2)) * R2 * tp2)].append((u + 1, k % G2, k // G2))

            def p2_body(sx_prev, sx_cur, s_cur, s_next, so_prev, so_cur, pin):
                parts = {}
                M = {}
                for z in range(U2 * R2):
                    u, r = divmod(z, R2)
                    if u == 0:
                        lhs = [a2buf[r, q] for q in range(G2)]
                    else:
                        lhs = [jnp.concatenate([parts[u, q, t][r] for t in range(nt2)], axis=0) for q in range(G2)]
                    M[u, r] = jnp.dot(jnp.concatenate(lhs, axis=1), pltpu.bitcast(b2[r], bf16), preferred_element_type=f32)
                    for k in range(tp2):
                        if u == U2 - 1:
                            m2buf[r, k * ST2:(k + 1) * ST2, :] = M[u, r][k * ST2:(k + 1) * ST2]
                        for (pu, t, c) in ot_at[z * tp2 + k]:
                            rows = slice(t * MT2, (t + 1) * MT2)
                            if xs2:
                                xbuf[pin, TM:TM + 16, 0:L] = M[u, r][k * ST2:k * ST2 + 16].astype(bf16)
                            if c:
                                out_tile(lambda v: m2buf[v, rows, :], sx_prev, so_prev, pu * CM2 + t * MT2)
                            else:
                                out_tile(lambda v: M[pu, v][rows], sx_cur, so_cur, pu * CM2 + t * MT2)
                        for (nu, q, t) in cb_at[z * tp2 + k]:
                            if hsync:
                                hbuf[pin, HS:HS + 16, :] = M[u, r][k * ST2:k * ST2 + 16].astype(bf16)
                            if nu < U2:
                                parts[nu, q, t] = comb_tile(s_cur, nu * CM2 + t * MT2, q)
                            else:
                                for r2, val in enumerate(comb_tile(s_next, t * MT2, q)):
                                    a2buf[r2, q, t * MT2:(t + 1) * MT2, :] = val

            def pro2(t, _):
                r0 = pl.multiple_of(t * MT2, MT2)
                for q in range(G2):
                    for r, val in enumerate(comb_tile(int(tab[4, 0]), r0, q)):
                        a2buf[r, q, pl.ds(r0, MT2), :] = val
            lax.fori_loop(0, nt2, pro2, None)

            def p2(j, _):
                jn = jnp.minimum(j + 1, T - 1)
                jd = jnp.minimum(j + D, T - 1)
                jp = jnp.maximum(j - 1, 0)

                @pl.when(jnp.logical_and(j + 1 < T, tab_ref[5, jn] >= 0))
                def _():
                    hr_copy(tab_ref[5, jn], tab_ref[4, jn]).wait()
                x_copy(tab_ref[3, j], lax.rem(j, NX)).wait()

                @pl.when(j >= NO)
                def _():
                    o_copy(tab_ref[3, jnp.maximum(j - NO, 0)], lax.rem(j, NO)).wait()
                if delay: pl.delay(delay)
                else: p2_body(lax.rem(jp, NX), lax.rem(j, NX), tab_ref[4, j], tab_ref[4, jn], lax.rem(j + NO - 1, NO), lax.rem(j, NO), zero[0])

                if not xfirst:
                    @pl.when(j >= 1)
                    def _():
                        o_copy(tab_ref[3, jp], lax.rem(jp, NO)).start(priority=po)
                @pl.when(j - 1 + NX < T)
                def _():
                    x_copy(tab_ref[3, jnp.minimum(j - 1 + NX, T - 1)], lax.rem(j - 1 + NX, NX)).start(priority=px)

                if xfirst:
                    @pl.when(j >= 1)
                    def _():
                        o_copy(tab_ref[3, jp], lax.rem(jp, NO)).start(priority=po)
                @pl.when(jnp.logical_and(j + D < T, tab_ref[5, jd] >= 0))
                def _():
                    hr_copy(tab_ref[5, jd], tab_ref[4, jd]).start(priority=ph)
            lax.fori_loop(0, T, p2, None)

            def epi2(t, _):
                r0 = pl.multiple_of(t * MT2, MT2)
                out_tile(lambda v: m2buf[v, pl.ds(r0, MT2), :], (T - 1) % NX, (T - 1) % NO, (U2 - 1) * CM2 + r0)
            lax.fori_loop(0, nt2, epi2, None)
            o_copy(int(tab[3, T - 1]), (T - 1) % NO).start(priority=po)
            for j in range(T - NO, T):
                o_copy(int(tab[3, j]), j % NO).wait()

        vm = pl.BlockSpec(memory_space=pltpu.VMEM)
        hb = pl.BlockSpec(memory_space=pl.ANY)
        out, _ = pl.pallas_call(
            kernel,
            in_specs=[pl.BlockSpec(memory_space=pltpu.SMEM), hb, vm, vm, vm, vm, vm],
            out_specs=[hb, hb],
            out_shape=[jax.ShapeDtypeStruct((N, C), bf16), jax.ShapeDtypeStruct((nsp, HS, L), bf16)],
            scratch_shapes=[
                pltpu.VMEM((NX, TM + 16, C), bf16), pltpu.VMEM((S, HS + 16, L), bf16), pltpu.VMEM((NO, TM, C), bf16),
                pltpu.VMEM((G1 * R1 + 2, L // 2, L), u32), pltpu.VMEM((R2 + 2, G2 * L // 2, L), u32),
                pltpu.VMEM((NT, 8, L), f32), pltpu.VMEM((8, C), f32), pltpu.SMEM((1,), jnp.int32), pltpu.VMEM((LN, C), f32), pltpu.VMEM((k1, nln * m1 * LT + 16, L), f32),
                pltpu.VMEM((R1 * RB1 // 2 + 16, L), u32), pltpu.VMEM((R1 * RB1 // 2 + 16, L), u32),
                pltpu.VMEM((R2, G2, RB2, L), bf16), pltpu.VMEM((R2, RB2, L), f32),
                pltpu.SemaphoreType.DMA((NX,)), pltpu.SemaphoreType.DMA((S,)), pltpu.SemaphoreType.DMA((NO,)),
            ] + [pltpu.VMEM((R1 * RB1 + 24, L), f32)] * MS,
            compiler_params=pltpu.CompilerParams(vmem_limit_bytes=vmem_mb * 1024 * 1024, flags=flags),
        )(tab, x.reshape(N, C), dw.reshape(1, C), w1, w2, grn_g.reshape(1, F), grn_b.reshape(1, F))
        return out.reshape(B, H, W, C)
    return fn


@jax.jit
def pallas_standalone__modern_conv_block_slak__vision_kernel(x, dw, w1, w2, grn_g, grn_b):
    return build(LN=16,lnlag=8,pj=0)(x, dw, w1, w2, grn_g, grn_b)
```

```python
import jax
import jax.numpy as jnp
import numpy as np
from jax import lax
import jax.experimental.pallas as pl
import jax.experimental.pallas.tpu as pltpu

_C0 = float(np.sqrt(2.0 / np.pi))
_C1 = _C0 * 0.044715
_A = _C1 ** (1.0 / 3.0)
_K0 = _C0 / _A
_GS = 0.5 / _A


def lincomb(terms, get):
    pos = [v for v, c in terms if c > 0]
    neg = [v for v, c in terms if c < 0]
    sign = 1
    if not pos:
        pos, neg, sign = neg, [], -1
    acc = get(pos[0])
    for v, c in terms:
        if v == pos[0]:
            continue
        acc = acc + get(v) if c * sign > 0 else acc - get(v)
    return acc, sign


class Lazy:
    def __init__(self, nin, steps, leaf):
        self.nin, self.steps, self.leaf, self.memo = nin, steps, leaf, {}
    def __call__(self, v):
        if v not in self.memo:
            if v < self.nin:
                self.memo[v] = self.leaf(v)
            else:
                i, j, s = self.steps[v - self.nin]
                self.memo[v] = self(i) + self(j) if s > 0 else self(i) - self(j)
        return self.memo[v]


def cse(rows):
    R = [list(map(int, r)) for r in rows]; steps = []
    while True:
        n = len(R[0]); best = 1; arg = None
        for i in range(n):
            for j in range(i+1, n):
                a = sum(1 for r in R if r[i]*r[j] > 0); b = sum(1 for r in R if r[i]*r[j] < 0)
                if a > best: best = a; arg = (i, j, 1)
                if b > best: best = b; arg = (i, j, -1)
        if arg is None: break
        i, j, s = arg; steps.append(arg)
        for r in R:
            if r[i]*r[j] == s: r.append(r[i]); r[i] = 0; r[j] = 0
            else: r.append(0)
    return steps, [[(v, c) for v, c in enumerate(r) if c] for r in R]

SCHEMES = {
    'fg/p233_2.txt': ((2, 3, 3), [[0, 0, 0, 0, 0, 1], [1, 0, 0, -1, 1, 0], [0, -1, -1, 0, 0, 1], [1, 0, 1, 0, 0, 0], [0, 0, 0, -1, 0, -1], [-1, 0, 0, 0, 0, -1], [0, 1, 0, 0, 0, 0], [0, 0, 1, 0, 0, -1], [-1, 0, 0, 0, 0, 0], [0, -1, -1, 0, 1, 1], [0, 0, 0, 0, 1, 0], [-1, 1, 0, 1, -1, 0], [0, 0, 0, 1, -1, 0], [0, -1, -1, 0, 0, 0], [1, 0, 0, -1, 0, 0]], [[1, 0, 1, 0, 0, 0, -1, 0, 0], [0, 0, -1, 0, -1, 0, 0, 0, 0], [0, 0, 0, -1, 0, -1, 0, 0, 1], [0, 0, 0, 0, 0, 0, 0, -1, 0], [-1, 0, -1, 0, 0, 0, 0, 0, 0], [1, 0, 1, 0, 0, 0, 0, -1, 0], [0, 0, 0, 0, -1, 1, 0, 0, -1], [0, 0, 0, -1, 0, -1, 1, -1, 1], [0, 1, -1, 0, 0, 0, 0, -1, 0], [0, 0, 0, 1, 0, 1, 0, 0, 0], [0, 0, -1, 1, 0, 0, 0, 0, 0], [0, 0, 0, 0, 1, 0, 0, 0, 0], [0, 0, 1, 0, 0, 0, 0, 0, 0], [0, 0, 0, 0, 0, 0, 0, 0, -1], [-1, 1, -1, 0, 1, 0, 0, 0, 0]], [[-1, 0, 0, -1, 0, 0], [1, -1, -1, 0, -1, 0], [1, 0, 0, 0, 0, 1], [-1, -1, 0, 0, 0, 0], [0, 0, 0, 1, 1, 0], [-1, 0, 0, 0, 1, 0], [-1, 0, 1, 0, 0, 0], [1, 0, 0, 0, 0, 0], [0, -1, 0, 0, -1, 0], [0, 0, 0, 0, 0, 1], [0, 0, 0, 1, 0, -1], [-1, 1, 1, 0, 0, 0], [-1, 1, 1, -1, 1, 1], [0, 0, 1, 0, 0, 1], [0, 0, 0, 0, -1, 0]]),
    'fg/p233_4.txt': ((2, 3, 3), [[0, 0, 0, 0, 0, -1], [-1, -1, 0, -1, -1, 0], [1, 0, 1, 0, 0, 0], [1, 0, 0, 0, 0, 0], [0, 0, 0, 0, 1, 0], [-1, -1, 0, 0, 0, -1], [1, 1, 0, 0, 1, 0], [0, 0, 0, -1, 0, 0], [0, 0, -1, 0, 0, -1], [0, 1, 0, 0, 1, 0], [-1, 0, -1, 0, 0, -1], [-1, -1, 1, 0, 0, 0], [-1, 0, -1, -1, 0, -1], [0, 0, 0, 1, 1, -1], [-1, -1, 0, 0, 0, 0]], [[0, 0, 0, -1, 0, 0, -1, 1, 0], [0, 0, 1, 1, 0, 0, 0, 0, 0], [0, 0, 0, 0, 0, 0, 0, -1, 0], [0, 1, -1, 0, -1, 1, 0, -1, 0], [0, 0, 0, 0, -1, 0, 0, 0, 0], [0, 0, 0, -1, 0, 0, 0, 0, 1], [0, 0, -1, 0, -1, 1, 0, 0, 0], [-1, 1, 0, 1, 0, 0, 0, 0, 0], [-1, 0, 0, 1, 0, 0, 1, 0, 1], [0, 0, 1, 0, 0, -1, 0, 0, 0], [1, 0, 0, -1, 0, 0, 0, -1, 0], [0, 0, 0, 0, 0, 0, 0, 0, -1], [-1, 0, 0, 1, 0, 0, 0, 0, 0], [0, 0, 0, 1, 0, 0, 0, 0, 0], [0, 0, 0, 0, -1, 1, 0, 0, 1]], [[-1, 0, 0, 1, 0, 0], [0, 0, 0, 0, 0, -1], [-1, -1, 0, 1, 1, 0], [0, 1, 0, 0, 0, 0], [0, 1, 1, 0, -1, -1], [1, 0, 0, 0, 0, -1], [0, -1, -1, 0, 0, 1], [0, 0, 0, 0, -1, 0], [-1, 0, 0, 0, 0, 0], [0, -1, -1, 0, 0, 0], [-1, 0, 0, 1, 1, 0], [1, 0, -1, 0, 0, 0], [0, 0, 0, 1, 1, 0], [0, 0, 0, 1, 0, -1], [0, 0, -1, 0, 0, 1]]),
}


def load_scheme(name):
    sh, U, V, W = SCHEMES[name]
    return sh, np.array(U), np.array(V), np.array(W)

def schedule(T, S, NS, D):
    spread = S - NS
    keep = [((i + 1) * spread) // (T - NS) > (i * spread) // (T - NS) for i in range(T - NS)] + [True] * NS
    slot1, spill, wait1, last, nxt, rr, nsp = [], [], [], {}, NS, 0, 0
    for i in range(T):
        if keep[i] and i < T - NS:
            slot1.append(nxt); wait1.append(-1); nxt += 1
        else:
            slot1.append(rr); wait1.append(last.get(rr, -1)); last[rr] = i; rr = (rr + 1) % NS
        spill.append(-1 if keep[i] else nsp)
        nsp += not keep[i]
    kept = [i for i in range(T) if keep[i]][::-1]
    rest = [i for i in range(T) if not keep[i]]
    order, nk = kept[:D], len(kept) - D
    kept = kept[D:]
    for j in range(T - D):
        order.append(kept.pop(0) if ((j + 1) * nk) // (T - D) > (j * nk) // (T - D) else rest.pop(0))
    slot2 = []
    for j, i in enumerate(order):
        slot2.append(slot1[i] if keep[i] else slot2[j - D])
    src2 = [spill[i] for i in order]
    wsp = [spill[w] if w >= 0 else -1 for w in wait1]
    return np.array([slot1, spill, wsp, order, slot2, src2], np.int32), nsp


def fold_triangles(W):
    R = len(W)
    tri = [(p, q, r, a, b) for p in range(R) for q in range(p + 1, R) for r in range(R) for a in (1, -1) for b in (1, -1)
           if r != p and r != q and (W[r] == a * W[p] + b * W[q]).all()]
    def cost(sel):
        keep = [i for i in range(R) if i not in [t[2] for t in sel]]
        steps, outs = cse(W[keep].T)
        return 2 * len(sel) + len(steps) + sum(len(t) - 1 for t in outs)
    level, best = [()], ()
    while level:
        best = min(level, key=cost)
        level = [sel + (t,) for sel in level for t in tri
                 if (not sel or t > sel[-1]) and not set(t[:3]) & set(i for u in sel for i in u[:3])]
    return best


L = 128
NM = 4


def build(RB1=256, U1=2, RB2=128, U2=4, NX=4, NO=3, S=36, NS=4, D=5, vmem_mb=128, phase=3, dma=True,
          s1='fg/p233_4.txt', s2='fg/p233_2.txt', flags=None, pad=8,
          ST=16, lag1=12, gd=3, pj=0, lnlo=0.0, lnhi=0.9, lnlag=8, nln=4, pmode=8, mdel=4, pdel=2, LN=8,
          ST2=32, lag2=1, cblo=0.0, cbhi=0.9, cd=0, cprobe=0, xs2=True, mprobe=0, gpin=1, goff=-1, gdep=True, apin=True, xpin=0):
    def fn(x, dw, w1, w2, grn_g, grn_b):
        B, H, W, C = x.shape
        F = w1.shape[1]
        N = B * H * W
        f32, bf16, u32 = jnp.float32, jnp.bfloat16, jnp.uint32
        (m1, k1, n1), Us1, Vs1, Ws1 = load_scheme(s1)
        (m2, k2, n2), Us2, Vs2, Ws2 = load_scheme(s2)
        R1, R2 = len(Us1), len(Us2)
        assert k1 * L == C and n2 * L == C
        G1, G2 = F // (n1 * L), F // (k2 * L)
        a1_steps, a1_out = cse(Us1)
        tris = fold_triangles(Ws1)
        kept1 = [r for r in range(R1) if r not in [t[2] for t in tris]]
        K1 = len(kept1)
        c1_steps, c1_out = cse(Ws1[kept1].T)
        loose = [r for r in range(R1) if r not in [i for t in tris for i in t[:3]]]
        dots1, pend = [], [(list(tris), [(a, r) for r in loose]) for a in range(U1 * G1)]
        for a in range(U1 * G1):
            todo, free = pend[a]
            while todo or free:
                if todo and len(dots1) % NM <= 1 and (len(dots1) % NM == 1 or len(free) <= len(todo) or len(tris) < 4):
                    dots1 += [(a, r) for r in todo.pop(0)[:3]]
                else:
                    dots1.append((free or pend[a + 1][1]).pop(0))
        a2_steps, a2_out = cse(Us2)
        c2_steps, c2_out = cse(Ws2.T)
        sg1 = [1 if any(c > 0 for _, c in t) else -1 for t in a1_out]
        sg2 = [1 if any(c > 0 for _, c in t) else -1 for t in a2_out]
        direct2 = [len(t) == 1 and t[0][0] < m2 * k2 for t in a2_out]
        CM1, CM2 = m1 * RB1, m2 * RB2
        TM = CM1 * U1
        assert TM == CM2 * U2 and N % TM == 0 and U1 % 2 == 0 and U2 % 2 == 0 and (U1 * G1) % 4 == 0
        T, NT = N // TM, F // L
        tab, nsp = schedule(T, S, NS, D)
        M1R, A1R, M2R, A2R, HR = RB1 + pad, RB1 // 2 + pad, RB2 + pad, RB2 // 2 + pad, TM // 2 + pad
        HS = NT * HR
        BR = max(K1 * M1R, R2 * G2 * A2R)
        SR = max(K1 * M1R, R2 * M2R)
        AR = R1 * A1R
        LR = nln * m1 * 16
        pack = lambda lo, hi: pltpu.pack_elementwise([lo, hi], packed_dtype=bf16)
        unpack = lambda w, i: pltpu.unpack_elementwise(w, index=i, packed_dtype=bf16, unpacked_dtype=f32)
        as_u, as_f, as_b = (lambda v: pltpu.bitcast(v, u32)), (lambda v: pltpu.bitcast(v, f32)), (lambda v: pltpu.bitcast(v, bf16))

        def kernel(tab_ref, x_hbm, dw_ref, w1_hbm, w2_hbm, g_ref, b_ref, o_hbm, h_hbm,
                   xbuf, hbuf, obuf, wbuf, acc, row, zero, lnbuf, a1e, a1o, big0, big1, sm0, sm1, xsem, hsem, osem, wsem):
            a1b, mbs, a2b, m2b = (a1e, a1o), (big0, big1, sm0, sm1), (big0, big1), (sm0, sm1)
            mtail = (BR, BR, SR, SR)

            class _Nop:
                def start(self): pass
                def wait(self): pass
            mk = pltpu.make_async_copy if dma else (lambda *a: _Nop())
            def x_copy(i, s): return mk(x_hbm.at[pl.ds(i * TM, TM)], xbuf.at[s, pl.ds(0, TM)], xsem.at[s])
            def hw_copy(i, s): return mk(hbuf.at[s, pl.ds(0, HS)], h_hbm.at[i], hsem.at[s])
            def hr_copy(i, s): return mk(h_hbm.at[i], hbuf.at[s, pl.ds(0, HS)], hsem.at[s])
            def o_copy(i, s): return mk(obuf.at[s], o_hbm.at[pl.ds(i * TM, TM)], osem.at[s])

            w1_copies = [pltpu.make_async_copy(w1_hbm.at[:, pl.ds(c * C, C)], obuf.at[c // 2, pl.ds((c % 2) * C, C)], wsem.at[c])
                         for c in range(4)]
            w2_copies = [pltpu.make_async_copy(w2_hbm.at[pl.ds(r0, n)], obuf.at[s, pl.ds(d0, n)], wsem.at[4 + s])
                         for r0, n, s, d0 in ((0, 8 * L, 2, 0), (8 * L, 2 * L, 0, 2 * C), (10 * L, 2 * L, 1, 2 * C))]
            def w1_tile(kt, ct):
                c, j = divmod(ct, C // L)
                return obuf[c // 2, (c % 2) * C + kt * L:(c % 2) * C + (kt + 1) * L, j * L:(j + 1) * L].astype(f32)
            def w2_tile(ct, j):
                s, r0 = (2, ct * L) if ct < 8 else ((ct - 8) // 2, 2 * C + ((ct - 8) % 2) * L)
                return obuf[s, r0:r0 + L, j * L:(j + 1) * L].astype(f32)

            for cp in w1_copies:
                cp.start()
            for j in range(NX):
                x_copy(j, j).start()
            for cp in w2_copies:
                cp.start()
            zero[0] = 0
            acc[...] = jnp.zeros_like(acc)
            for buf, t in zip(mbs + a1b, mtail + (AR, AR)):
                buf[t:t + 24, :] = jnp.zeros((24, L), buf.dtype)
            row[0] = jnp.broadcast_to(dw_ref[...].astype(f32), (8, C))

            def ln_store(s, r0, lrow):
                o = xbuf[s, pl.ds(r0, LN), :].astype(f32) * jnp.concatenate([row[0]] * (LN // 8), axis=0)
                mu = jnp.sum(o, axis=-1, keepdims=True) * (1.0 / C)
                d = o - mu
                v = jnp.sum(d * d, axis=-1, keepdims=True) * (1.0 / C)
                a = d * (lax.rsqrt(v + 1e-5) * _A)
                for j in range(k1):
                    lnbuf[j, pl.ds(lrow, LN), :] = a[:, j * L:(j + 1) * L]

            def ac_tile(lrow, dst, drow):
                halves = []
                for par in range(2):
                    av = Lazy(m1 * k1, a1_steps, lambda v: lnbuf[v % k1, pl.ds(lrow + (v // k1) * 16 + par, 8, stride=2), :])
                    halves.append([lincomb(a1_out[r], av)[0] for r in range(R1)])
                for r in range(R1):
                    dst[pl.ds(drow + r * A1R, 8), :] = pack(halves[0][r], halves[1][r])

            def gelu_rows(getm, g, sq):
                mv = Lazy(K1, c1_steps, getm)
                res = []
                for e in range(m1 * n1):
                    y, sg = lincomb(c1_out[e], mv)
                    th = jnp.tanh(y * (y * y + _K0))
                    hv = y * (th + 1.0) if sg > 0 else y * (th - 1.0)
                    ct = (e % n1) * G1 + g
                    sq[ct] = sq[ct] + hv * hv if ct in sq else hv * hv
                    res.append(hv)
                return res

            def h_store(lo, hi, s, r0, g):
                for e in range(m1 * n1):
                    hbuf[s, pl.ds(r0 + ((e % n1) * G1 + g) * HR + (e // n1) * (RB1 // 2), 8), :] = pack(lo[e], hi[e])

            def flush_sq(sq):
                for ct in sorted(sq):
                    acc[ct] += sq[ct]
                sq.clear()

            tpr = RB1 // ST
            ntick = len(dots1) // NM * tpr
            nt = RB1 // 8
            ge_at = [[] for _ in range(ntick)]
            for a in range(U1 * G1):
                ready = (max(z for z, d in enumerate(dots1) if d[0] == a) // NM + 1) * tpr
                for t in range(nt):
                    z = max(((a + 1) * R1 * tpr) // NM + lag1 + (t * R1 * tpr) // (NM * nt), ready)
                    if t % 2 and z >= ntick > zprev:
                        z = ntick - 1
                    zprev = z
                    ge_at[z % ntick].append((a, t, z >= ntick))
            carried = sorted({(a, t) for ev in ge_at for a, t, c in ev if c})
            per16 = m1 * (16 // LN)
            ln_at, ac_at = [[] for _ in range(ntick)], [[] for _ in range(ntick)]
            for u in range(U1):
                n_it = RB1 // 16 * per16
                for it in range(n_it):
                    z = int((u + lnlo + (lnhi - lnlo) * it / n_it) * ntick / U1)
                    ln_at[z].append((u + 1, it // per16, it % per16))
                    if (it + 1) % per16 == 0:
                        ac_at[z + lnlag].append((u + 1, it // per16))

            def p1_body(s_prev, s_cur, sx_cur, sx_next, zp):
                z0 = pl.multiple_of(zero[0], 8)
                sq, held, done, probes = {}, [], [], []
                for rho in range(len(dots1) // NM):
                    res = []
                    for a, r in dots1[rho * NM:(rho + 1) * NM]:
                        lhs = as_b(a1b[(a // G1) % 2][r * A1R:r * A1R + RB1 // 2, :])
                        res.append((a, r, jnp.dot(lhs, as_b(wbuf[(a % G1) * R1 + r]), preferred_element_type=f32)))
                    for k in range(tpr):
                        pv = res[pj][2][k * ST:k * ST + 8]
                        got = {(a, r): val[k * ST:(k + 1) * ST] for a, r, val in res}
                        for p, q, r, ca, cb in tris:
                            for a in sorted({a for a, r2 in got if r2 == r}):
                                m = got.pop((a, r))
                                got[a, p] = got[a, p] + m if ca > 0 else got[a, p] - m
                                got[a, q] = got[a, q] + m if cb > 0 else got[a, q] - m
                        for (a, r), val in got.items():
                            mbs[a % 4][pl.ds(z0 + kept1.index(r) * M1R, ST) if k == 0 else pl.ds(z0 + kept1.index(r) * M1R + k * ST, ST), :] = val
                        if k % pmode == pmode - 1:
                            for a in sorted({a for a, _, _ in res}):
                                probes.append((len(done) + mdel, mbs[a % 4][mtail[a % 4] + 16:mtail[a % 4] + 24, :]))
                            probes.sort(key=lambda e: e[0])
                        for (pa, t, c) in ge_at[rho * tpr + k]:
                            pu, pg = divmod(pa, G1)
                            val = pv
                            if len(done) >= gd:
                                val = done[-gd] + pv
                                while probes and probes[0][0] <= len(done):
                                    val = val + probes.pop(0)[1]
                            if gpin and t % gpin == goff % gpin:
                                mbs[pa % 4][pl.ds(mtail[pa % 4] + zp, 8), :] = val if gdep else pv
                            held.append(gelu_rows(lambda v: mbs[pa % 4][v * M1R + t * 8:v * M1R + (t + 1) * 8, :], pg, sq))
                            done.append(sum([sq[l * G1 + pg] for l in range(1, n1)], sq[pg]))
                            if len(held) == 2:
                                h_store(held[0], held[1], s_prev if c else s_cur, (pu * CM1 + (t - 1) * 8) // 2, pg)
                                held = []
                            if t == nt - 1:
                                flush_sq(sq)
                        for (nu, t, j) in ln_at[rho * tpr + k]:
                            if xpin:
                                xbuf[z0, TM:TM + 8, 0:L] = pv.astype(bf16)
                            q, j2 = divmod(j, 16 // LN)
                            ln_store(sx_cur if nu < U1 else sx_next, (nu % U1) * CM1 + q * RB1 + t * 16 + j2 * LN,
                                     z0 + (t % nln) * m1 * 16 + j * LN)
                        for (nu, t) in ac_at[rho * tpr + k]:
                            if apin:
                                lnbuf[0, pl.ds(LR + zp, 8), :] = pv
                            ac_tile((t % nln) * m1 * 16, a1b[nu % 2], z0 + t * 8)
                            probes.append((len(done) + pdel, as_f(a1b[nu % 2][AR:AR + 8, :])))
                flush_sq(sq)

            for a in sorted({a % 4 for a, _ in carried}):
                mbs[a][0:K1 * M1R, :] = jnp.zeros((K1 * M1R, L), f32)
            for cp in w1_copies:
                cp.wait()
            for g in range(G1):
                for r in range(R1):
                    val, sg = lincomb([(v, int(c) * sg1[r]) for v, c in enumerate(Vs1[r]) if c],
                                      lambda v: w1_tile(v // n1, (v % n1) * G1 + g))
                    wbuf[g * R1 + r] = as_u((val if sg > 0 else -val).astype(bf16))

            if phase & 1:
                x_copy(0, 0).wait()

                def pro(t, _):
                    for j in range(per16):
                        q, j2 = divmod(j, 16 // LN)
                        ln_store(0, pl.multiple_of(t * 16, 16) + q * RB1 + j2 * LN, j * LN)
                    ac_tile(0, a1e, pl.multiple_of(t * 8, 8))
                lax.fori_loop(0, RB1 // 16, pro, None)

                def p1(i, _):
                    ip = jnp.maximum(i - 1, 0)

                    @pl.when(i + 1 < T)
                    def _():
                        x_copy(i + 1, lax.rem(i + 1, NX)).wait()

                    @pl.when(tab_ref[2, i] >= 0)
                    def _():
                        hw_copy(tab_ref[2, i], tab_ref[0, i]).wait()
                    p1_body(jnp.where(i > 0, tab_ref[0, ip], S - 1), tab_ref[0, i], lax.rem(i, NX), lax.rem(jnp.minimum(i + 1, T - 1), NX),
                            pl.multiple_of(8 * lax.rem(i, 2), 8))

                    @pl.when(i + NX < T)
                    def _():
                        x_copy(i + NX, lax.rem(i, NX)).start()

                    @pl.when(jnp.logical_and(i >= 1, tab_ref[1, ip] >= 0))
                    def _():
                        hw_copy(tab_ref[1, ip], tab_ref[0, ip]).start()
                lax.fori_loop(0, T, p1, None)
                if phase & 2:
                    for j in range(NX - 1):
                        x_copy(int(tab[3, j]), j).start()
                for a in sorted({a for a, _ in carried}):
                    def epi(t, _):
                        sq = {}
                        r0 = pl.multiple_of(t * 16, 16)
                        lo, hi = (gelu_rows(lambda v: mbs[a % 4][pl.ds(v * M1R + r0 + 8 * i, 8), :], a % G1, sq) for i in range(2))
                        h_store(lo, hi, int(tab[0, T - 1]), pl.multiple_of(t * 8, 8) + (a // G1) * CM1 // 2, a % G1)
                        flush_sq(sq)
                    lax.fori_loop(min(t for ca, t in carried if ca == a) // 2, nt // 2, epi, None)
            else:
                for j in range(NX):
                    x_copy(j, j).wait()
                for j in range(NX - 1):
                    x_copy(j, j).start()
            for cp in w2_copies:
                cp.wait()
            if not (phase & 2):
                return

            ss = jnp.concatenate([jnp.sum(acc[c], axis=0, keepdims=True) for c in range(NT)], axis=1) * (_GS * _GS)
            gx = jnp.sqrt(ss + 1e-6)
            nx = gx / (jnp.sum(gx, axis=-1, keepdims=True) * (1.0 / F) + 1e-6)
            sc = (g_ref[...].astype(f32) * nx + 1.0) * _GS
            sct = jnp.transpose(jnp.broadcast_to(sc, (L, F)))
            bt = jnp.transpose(jnp.broadcast_to(b_ref[...].astype(f32), (L, F)))
            for q in range(G2):
                for r in range(R2):
                    def get(v):
                        ct = (v // n2) * G2 + q
                        return w2_tile(ct, v % n2) * sct[ct * L:(ct + 1) * L]
                    val, sg = lincomb([(v, int(c) * sg2[r]) for v, c in enumerate(Vs2[r]) if c], get)
                    wbuf[r * G2 + q] = as_u((val if sg > 0 else -val).astype(bf16))
            for j in range(n2):
                p = sum(w2_tile(ct, j) * bt[ct * L:(ct + 1) * L] for ct in range(NT))
                row[1, :, j * L:(j + 1) * L] = jnp.broadcast_to(jnp.sum(p, axis=0, keepdims=True), (8, L))
            sm1[0:R2 * M2R, :] = jnp.zeros((R2 * M2R, L), f32)

            def comb_tile(s, r0, q, dst, drow):
                raw = Lazy(m2 * k2, [], lambda v: hbuf[s, pl.ds(r0 + ((v % k2) * G2 + q) * HR + (v // k2) * (RB2 // 2), 8), :])
                avs = [Lazy(m2 * k2, a2_steps, lambda v, i=i: unpack(raw(v), i)) for i in range(2)]
                for r in range(R2):
                    dst[pl.ds(drow + (r * G2 + q) * A2R, 8), :] = as_f(
                        raw(a2_out[r][0][0]) if direct2[r] else pack(*(lincomb(a2_out[r], av)[0] for av in avs)))

            def out_tile(src, srow, sx, so, r0):
                mvs = [Lazy(R2, c2_steps, lambda v, i=i: src[pl.ds(srow + v * M2R + i, 8, stride=2), :]) for i in range(2)]
                for i in range(m2):
                    rows = pl.ds(r0 + i * RB2, 16)
                    xv = xbuf[sx, rows, :].astype(f32) + jnp.concatenate([row[1]] * 2, axis=0)
                    res = []
                    for l in range(n2):
                        ys = [lincomb(c2_out[i * n2 + l], mv) for mv in mvs]
                        y, z = jnp.concatenate([ys[0][0], ys[1][0]], axis=0), xv[:, l * L:(l + 1) * L]
                        res.append(z + y if ys[0][1] > 0 else z - y)
                    obuf[so, rows, :] = jnp.concatenate(res, axis=1).astype(bf16)

            tp2 = RB2 // ST2
            ntick2 = U2 * R2 * tp2
            nt2 = RB2 // 16
            ot_at, cb_at = [[] for _ in range(ntick2)], [[] for _ in range(ntick2)]
            for u in range(U2):
                for t in range(nt2):
                    z = (u + 1) * R2 * tp2 + lag2 + (t * (R2 * tp2 - lag2)) // nt2
                    ot_at[z % ntick2].append((u, t, z >= ntick2))
                for k in range(G2 * nt2):
                    cb_at[int((u + cblo + (cbhi - cblo) * k / (G2 * nt2)) * R2 * tp2)].append((u + 1, k % G2, k // G2))

            def p2_body(sx_prev, sx_cur, s_cur, s_next, so_prev, so_cur):
                z0 = pl.multiple_of(zero[0], 8)
                probes, ncb = [], 0
                for z in range(U2 * R2):
                    u, r = divmod(z, R2)
                    ys = [jnp.dot(as_b(a2b[u % 2][(r * G2 + q) * A2R:(r * G2 + q) * A2R + RB2 // 2, :]), as_b(wbuf[r * G2 + q]),
                                  preferred_element_type=f32) for q in range(G2)]
                    val = (ys[0] + ys[1]) + (ys[2] + ys[3])
                    for k in range(tp2):
                        pv = val[k * ST2:k * ST2 + 8]
                        m2b[u % 2][pl.ds(z0 + r * M2R + k * ST2, ST2), :] = val[k * ST2:(k + 1) * ST2]
                        if mprobe and k == tp2 - 1:
                            probes.append((ncb + mprobe, m2b[u % 2][SR + 8:SR + 16, :]))
                            probes.sort(key=lambda e: e[0])
                        for (pu, t, c) in ot_at[z * tp2 + k]:
                            m2b[pu % 2][pl.ds(z0 + SR, 8), :] = pv
                            if xs2:
                                xbuf[z0, TM:TM + 8, 0:L] = pv.astype(bf16)
                            out_tile(m2b[pu % 2], t * 16, sx_prev if c else sx_cur, so_prev if c else so_cur, pu * CM2 + t * 16)
                        for (nu, q, t) in cb_at[z * tp2 + k]:
                            pin = pv
                            while probes and probes[0][0] <= ncb:
                                pin = pin + probes.pop(0)[1]
                            hbuf[z0, HS:HS + 8, :] = as_u(pin)
                            comb_tile(s_cur if nu < U2 else s_next, ((nu % U2) * CM2 + t * 16) // 2, q, a2b[nu % 2], z0 + t * 8)
                            ncb += 1
                            if cprobe and ncb % cprobe == 0:
                                probes.append((ncb + cd, a2b[nu % 2][BR + 8:BR + 16, :]))
                                probes.sort(key=lambda e: e[0])

            def pro2(t, _):
                r0 = pl.multiple_of(t * 8, 8)
                for q in range(G2):
                    comb_tile(int(tab[4, 0]), r0, q, big0, r0)
            lax.fori_loop(0, nt2, pro2, None)

            def p2(j, _):
                jn, jd, jp = jnp.minimum(j + 1, T - 1), jnp.minimum(j + D, T - 1), jnp.maximum(j - 1, 0)

                @pl.when(jnp.logical_and(j + 1 < T, tab_ref[5, jn] >= 0))
                def _():
                    hr_copy(tab_ref[5, jn], tab_ref[4, jn]).wait()
                x_copy(tab_ref[3, j], lax.rem(j, NX)).wait()

                @pl.when(j >= NO)
                def _():
                    o_copy(tab_ref[3, jnp.maximum(j - NO, 0)], lax.rem(j, NO)).wait()
                p2_body(lax.rem(jp, NX), lax.rem(j, NX), tab_ref[4, j], tab_ref[4, jn], lax.rem(j + NO - 1, NO), lax.rem(j, NO))

                @pl.when(j >= 1)
                def _():
                    o_copy(tab_ref[3, jp], lax.rem(jp, NO)).start()

                @pl.when(j - 1 + NX < T)
                def _():
                    x_copy(tab_ref[3, jnp.minimum(j - 1 + NX, T - 1)], lax.rem(j - 1 + NX, NX)).start()

                @pl.when(jnp.logical_and(j + D < T, tab_ref[5, jd] >= 0))
                def _():
                    hr_copy(tab_ref[5, jd], tab_ref[4, jd]).start()
            lax.fori_loop(0, T, p2, None)

            def epi2(t, _):
                r0 = pl.multiple_of(t * 16, 16)
                out_tile(sm1, r0, (T - 1) % NX, (T - 1) % NO, (U2 - 1) * CM2 + r0)
            lax.fori_loop(0, nt2, epi2, None)
            o_copy(int(tab[3, T - 1]), (T - 1) % NO).start()
            for j in range(T - NO, T):
                o_copy(int(tab[3, j]), j % NO).wait()

        vm = pl.BlockSpec(memory_space=pltpu.VMEM)
        hb = pl.BlockSpec(memory_space=pl.ANY)
        out, _ = pl.pallas_call(
            kernel,
            in_specs=[pl.BlockSpec(memory_space=pltpu.SMEM), hb, vm, hb, hb, vm, vm],
            out_specs=[hb, hb],
            out_shape=[jax.ShapeDtypeStruct((N, C), bf16), jax.ShapeDtypeStruct((nsp, HS, L), u32)],
            scratch_shapes=[
                pltpu.VMEM((NX, TM + 16, C), bf16), pltpu.VMEM((S, HS + 8, L), u32), pltpu.VMEM((NO, TM, C), bf16),
                pltpu.VMEM((max(G1 * R1, G2 * R2), L // 2, L), u32), pltpu.VMEM((NT, 8, L), f32), pltpu.VMEM((2, 8, C), f32),
                pltpu.SMEM((1,), jnp.int32), pltpu.VMEM((k1, LR + 16, L), f32),
                pltpu.VMEM((AR + 24, L), u32), pltpu.VMEM((AR + 24, L), u32),
                pltpu.VMEM((BR + 24, L), f32), pltpu.VMEM((BR + 24, L), f32),
                pltpu.VMEM((SR + 24, L), f32), pltpu.VMEM((SR + 24, L), f32),
                pltpu.SemaphoreType.DMA((NX,)), pltpu.SemaphoreType.DMA((S,)), pltpu.SemaphoreType.DMA((NO,)),
                pltpu.SemaphoreType.DMA((7,)),
            ],
            compiler_params=pltpu.CompilerParams(vmem_limit_bytes=vmem_mb * 1024 * 1024, flags=flags),
        )(tab, x.reshape(N, C), dw.reshape(1, C), w1, w2, grn_g.reshape(1, F), grn_b.reshape(1, F))
        return out.reshape(B, H, W, C)
    return fn


@jax.jit
def pallas_standalone__modern_conv_block_slak__vision_kernel(x, dw, w1, w2, grn_g, grn_b):
    return build()(x, dw, w1, w2, grn_g, grn_b)
```

```python
import jax
import jax.numpy as jnp
import numpy as np
from jax import lax
import jax.experimental.pallas as pl
import jax.experimental.pallas.tpu as pltpu

L = 128
NM = 4

_C0 = float(np.sqrt(2.0 / np.pi))
_C1 = _C0 * 0.044715
_A = _C1 ** (1.0 / 3.0)
_K0 = _C0 / _A
_GS = 0.5 / _A


def _scheme(shape, products):
    m, k, n = shape
    U, V, W = (np.array([p[i] for p in products]) for i in range(3))
    want = np.zeros((m * k, k * n, m * n), int)
    for i in range(m):
        for j in range(k):
            for l in range(n):
                want[i * k + j, j * n + l, i * n + l] = 1
    assert (np.einsum("ra,rb,rc->abc", U, V, W) == want).all()
    return shape, U, V, W


SCHEME1 = _scheme((2, 3, 3), [
    ([0, 0, 0, 0, 0, -1], [0, 0, 0, -1, 0, 0, -1, 1, 0], [-1, 0, 0, 1, 0, 0]),
    ([-1, -1, 0, -1, -1, 0], [0, 0, 1, 1, 0, 0, 0, 0, 0], [0, 0, 0, 0, 0, -1]),
    ([1, 0, 1, 0, 0, 0], [0, 0, 0, 0, 0, 0, 0, -1, 0], [-1, -1, 0, 1, 1, 0]),
    ([1, 0, 0, 0, 0, 0], [0, 1, -1, 0, -1, 1, 0, -1, 0], [0, 1, 0, 0, 0, 0]),
    ([0, 0, 0, 0, 1, 0], [0, 0, 0, 0, -1, 0, 0, 0, 0], [0, 1, 1, 0, -1, -1]),
    ([-1, -1, 0, 0, 0, -1], [0, 0, 0, -1, 0, 0, 0, 0, 1], [1, 0, 0, 0, 0, -1]),
    ([1, 1, 0, 0, 1, 0], [0, 0, -1, 0, -1, 1, 0, 0, 0], [0, -1, -1, 0, 0, 1]),
    ([0, 0, 0, -1, 0, 0], [-1, 1, 0, 1, 0, 0, 0, 0, 0], [0, 0, 0, 0, -1, 0]),
    ([0, 0, -1, 0, 0, -1], [-1, 0, 0, 1, 0, 0, 1, 0, 1], [-1, 0, 0, 0, 0, 0]),
    ([0, 1, 0, 0, 1, 0], [0, 0, 1, 0, 0, -1, 0, 0, 0], [0, -1, -1, 0, 0, 0]),
    ([-1, 0, -1, 0, 0, -1], [1, 0, 0, -1, 0, 0, 0, -1, 0], [-1, 0, 0, 1, 1, 0]),
    ([-1, -1, 1, 0, 0, 0], [0, 0, 0, 0, 0, 0, 0, 0, -1], [1, 0, -1, 0, 0, 0]),
    ([-1, 0, -1, -1, 0, -1], [-1, 0, 0, 1, 0, 0, 0, 0, 0], [0, 0, 0, 1, 1, 0]),
    ([0, 0, 0, 1, 1, -1], [0, 0, 0, 1, 0, 0, 0, 0, 0], [0, 0, 0, 1, 0, -1]),
    ([-1, -1, 0, 0, 0, 0], [0, 0, 0, 0, -1, 1, 0, 0, 1], [0, 0, -1, 0, 0, 1]),
])
SCHEME2 = _scheme((2, 3, 3), [
    ([0, 0, 0, 0, 0, 1], [1, 0, 1, 0, 0, 0, -1, 0, 0], [-1, 0, 0, -1, 0, 0]),
    ([1, 0, 0, -1, 1, 0], [0, 0, -1, 0, -1, 0, 0, 0, 0], [1, -1, -1, 0, -1, 0]),
    ([0, -1, -1, 0, 0, 1], [0, 0, 0, -1, 0, -1, 0, 0, 1], [1, 0, 0, 0, 0, 1]),
    ([1, 0, 1, 0, 0, 0], [0, 0, 0, 0, 0, 0, 0, -1, 0], [-1, -1, 0, 0, 0, 0]),
    ([0, 0, 0, -1, 0, -1], [-1, 0, -1, 0, 0, 0, 0, 0, 0], [0, 0, 0, 1, 1, 0]),
    ([-1, 0, 0, 0, 0, -1], [1, 0, 1, 0, 0, 0, 0, -1, 0], [-1, 0, 0, 0, 1, 0]),
    ([0, 1, 0, 0, 0, 0], [0, 0, 0, 0, -1, 1, 0, 0, -1], [-1, 0, 1, 0, 0, 0]),
    ([0, 0, 1, 0, 0, -1], [0, 0, 0, -1, 0, -1, 1, -1, 1], [1, 0, 0, 0, 0, 0]),
    ([-1, 0, 0, 0, 0, 0], [0, 1, -1, 0, 0, 0, 0, -1, 0], [0, -1, 0, 0, -1, 0]),
    ([0, -1, -1, 0, 1, 1], [0, 0, 0, 1, 0, 1, 0, 0, 0], [0, 0, 0, 0, 0, 1]),
    ([0, 0, 0, 0, 1, 0], [0, 0, -1, 1, 0, 0, 0, 0, 0], [0, 0, 0, 1, 0, -1]),
    ([-1, 1, 0, 1, -1, 0], [0, 0, 0, 0, 1, 0, 0, 0, 0], [-1, 1, 1, 0, 0, 0]),
    ([0, 0, 0, 1, -1, 0], [0, 0, 1, 0, 0, 0, 0, 0, 0], [-1, 1, 1, -1, 1, 1]),
    ([0, -1, -1, 0, 0, 0], [0, 0, 0, 0, 0, 0, 0, 0, -1], [0, 0, 1, 0, 0, 1]),
    ([1, 0, 0, -1, 0, 0], [-1, 1, -1, 0, 1, 0, 0, 0, 0], [0, 0, 0, 0, -1, 0]),
])


def cse(rows):
    R = [list(map(int, r)) for r in rows]; steps = []
    while True:
        n = len(R[0]); best = 1; arg = None
        for i in range(n):
            for j in range(i+1, n):
                a = sum(1 for r in R if r[i]*r[j] > 0); b = sum(1 for r in R if r[i]*r[j] < 0)
                if a > best: best = a; arg = (i, j, 1)
                if b > best: best = b; arg = (i, j, -1)
        if arg is None: break
        i, j, s = arg; steps.append(arg)
        for r in R:
            if r[i]*r[j] == s: r.append(r[i]); r[i] = 0; r[j] = 0
            else: r.append(0)
    return steps, [[(v, c) for v, c in enumerate(r) if c] for r in R]


def lincomb(terms, get):
    pos = [v for v, c in terms if c > 0]
    neg = [v for v, c in terms if c < 0]
    sign = 1
    if not pos:
        pos, neg, sign = neg, [], -1
    acc = get(pos[0])
    for v, c in terms:
        if v == pos[0]:
            continue
        acc = acc + get(v) if c * sign > 0 else acc - get(v)
    return acc, sign


class Lazy:
    def __init__(self, nin, steps, leaf):
        self.nin, self.steps, self.leaf, self.memo = nin, steps, leaf, {}
    def __call__(self, v):
        if v not in self.memo:
            if v < self.nin:
                self.memo[v] = self.leaf(v)
            else:
                i, j, s = self.steps[v - self.nin]
                self.memo[v] = self(i) + self(j) if s > 0 else self(i) - self(j)
        return self.memo[v]


def schedule(T, S, NS, D):
    spread = S - NS
    keep = [((i + 1) * spread) // (T - NS) > (i * spread) // (T - NS) for i in range(T - NS)] + [True] * NS
    slot1, spill, wait1, last, nxt, rr, nsp = [], [], [], {}, NS, 0, 0
    for i in range(T):
        if keep[i] and i < T - NS:
            slot1.append(nxt); wait1.append(-1); nxt += 1
        else:
            slot1.append(rr); wait1.append(last.get(rr, -1)); last[rr] = i; rr = (rr + 1) % NS
        spill.append(-1 if keep[i] else nsp)
        nsp += not keep[i]
    kept = [i for i in range(T) if keep[i]][::-1]
    rest = [i for i in range(T) if not keep[i]]
    order, nk = kept[:D], len(kept) - D
    kept = kept[D:]
    for j in range(T - D):
        order.append(kept.pop(0) if ((j + 1) * nk) // (T - D) > (j * nk) // (T - D) else rest.pop(0))
    slot2 = []
    for j, i in enumerate(order):
        slot2.append(slot1[i] if keep[i] else slot2[j - D])
    src2 = [spill[i] for i in order]
    wsp = [spill[w] if w >= 0 else -1 for w in wait1]
    return np.array([slot1, spill, wsp, order, slot2, src2], np.int32), nsp


def fold_triangles(W):
    R = len(W)
    tri = [(p, q, r, a, b) for p in range(R) for q in range(p + 1, R) for r in range(R) for a in (1, -1) for b in (1, -1)
           if r != p and r != q and (W[r] == a * W[p] + b * W[q]).all()]
    def cost(sel):
        keep = [i for i in range(R) if i not in [t[2] for t in sel]]
        steps, outs = cse(W[keep].T)
        return 2 * len(sel) + len(steps) + sum(len(t) - 1 for t in outs)
    level, best = [()], ()
    while level:
        best = min(level, key=cost)
        level = [sel + (t,) for sel in level for t in tri
                 if (not sel or t > sel[-1]) and not set(t[:3]) & set(i for u in sel for i in u[:3])]
    return best


RB1 = 128
U1 = 4
RB2 = 64
U2 = 8
NX = 5
XA = 3
S = 38
NS = 4
D = 3
ST = 16
lag1 = 6
gd = 3
lnhi = 0.85
lnlag = 4
nln = 4
pmode = 4
mdel = 4
pdel = 2
LN = 8
ST2 = 32
lag2 = 1
cbhi = 0.8
cd = 2


@jax.jit
def pallas_standalone__modern_conv_block_slak__vision_kernel(x, dw, w1, w2, grn_g, grn_b):
    B, H, W, C = x.shape
    assert B == 1 and dw.shape[:2] == (1, 1)
    F = w1.shape[1]
    N = B * H * W
    f32, bf16, u32 = jnp.float32, jnp.bfloat16, jnp.uint32
    (m1, k1, n1), Us1, Vs1, Ws1 = SCHEME1
    (m2, k2, n2), Us2, Vs2, Ws2 = SCHEME2
    R1, R2 = len(Us1), len(Us2)
    assert k1 * L == C and n2 * L == C
    G1, G2 = F // (n1 * L), F // (k2 * L)
    a1_steps, a1_out = cse(Us1)
    tris = fold_triangles(Ws1)
    kept1 = [r for r in range(R1) if r not in [t[2] for t in tris]]
    K1 = len(kept1)
    c1_steps, c1_out = cse(Ws1[kept1].T)
    loose = [r for r in range(R1) if r not in [i for t in tris for i in t[:3]]]
    dots1, pend = [], [(list(tris), [(a, r) for r in loose]) for a in range(U1 * G1)]
    for a in range(U1 * G1):
        todo, free = pend[a]
        while todo or free:
            if todo and len(dots1) % NM <= 1 and (len(dots1) % NM == 1 or len(free) <= len(todo) or len(tris) < 4):
                dots1 += [(a, r) for r in todo.pop(0)[:3]]
            else:
                dots1.append((free or pend[a + 1][1]).pop(0))
    a2_steps, a2_out = cse(Us2)
    c2_steps, c2_out = cse(Ws2.T)
    sg1 = [1 if any(c > 0 for _, c in t) else -1 for t in a1_out]
    sg2 = [1 if any(c > 0 for _, c in t) else -1 for t in a2_out]
    direct2 = [len(t) == 1 and t[0][0] < m2 * k2 for t in a2_out]
    CM1, CM2 = m1 * RB1, m2 * RB2
    TM = CM1 * U1
    assert TM == CM2 * U2 and N % TM == 0 and U1 % 2 == 0 and U2 % 2 == 0 and (U1 * G1) % 4 == 0
    assert (CM2 // 2) % (RB1 // 2) == 0
    T, NT = N // TM, F // L
    tab, nsp = schedule(T, S, NS, D)
    M1R, A1R, M2R, A2R = RB1 + 8, RB1 // 2 + 8, RB2 + 8, RB2 // 2 + 8
    HC = CM2 // 2
    HS = NT * TM // 2
    hrow = lambda ct, r: (r // HC) * (NT * HC) + ct * HC + r % HC
    BR = max(K1 * M1R, R2 * G2 * A2R)
    SR = max(K1 * M1R, R2 * M2R)
    AR = R1 * A1R
    LR = nln * m1 * 16
    pack = lambda lo, hi: pltpu.pack_elementwise([lo, hi], packed_dtype=bf16)
    unpack = lambda w, i: pltpu.unpack_elementwise(w, index=i, packed_dtype=bf16, unpacked_dtype=f32)
    as_u, as_f, as_b = (lambda v: pltpu.bitcast(v, u32)), (lambda v: pltpu.bitcast(v, f32)), (lambda v: pltpu.bitcast(v, bf16))

    def kernel(tab_ref, x_hbm, dw_ref, w1_hbm, w2_hbm, g_ref, b_ref, o_hbm, h_hbm,
               xbuf, hbuf, wbuf, acc, row, zero, lnbuf, a1e, a1o, big0, big1, sm0, sm1, xsem, hsem, osem, wsem):
        a1b, mbs, a2b, m2b = (a1e, a1o), (big0, big1, sm0, sm1), (big0, big1), (sm0, sm1)
        mtail = (BR, BR, SR, SR)

        mk = pltpu.make_async_copy
        def x_copy(i, s): return mk(x_hbm.at[pl.ds(i * TM, TM)], xbuf.at[s, pl.ds(0, TM)], xsem.at[s])
        def hw_copy(i, s): return mk(hbuf.at[s, pl.ds(0, HS)], h_hbm.at[i], hsem.at[s])
        def hr_head(i, s): return mk(h_hbm.at[i, pl.ds(0, NT * HC)], hbuf.at[s, pl.ds(0, NT * HC)], hsem.at[s])
        def hr_rest(i, s): return mk(h_hbm.at[i, pl.ds(NT * HC, HS - NT * HC)], hbuf.at[s, pl.ds(NT * HC, HS - NT * HC)], hsem.at[S + s])
        def o_copy(i, s): return mk(xbuf.at[s, pl.ds(0, TM)], o_hbm.at[pl.ds(i * TM, TM)], osem.at[s])

        XO = (XA - (T - NX)) % NX
        xslot = lambda i: lax.rem(i + XO, NX)
        ws1, ws2 = [(NX - 2 + c + XO) % NX for c in range(2)], [XA, XA + 1]
        w1_copies = [pltpu.make_async_copy(w1_hbm.at[:, pl.ds(c * C, C)], xbuf.at[ws1[c // 2], pl.ds((c % 2) * C, C)], wsem.at[c])
                     for c in range(4)]
        w2_copies = [pltpu.make_async_copy(w2_hbm.at[pl.ds(c * 2 * C, 2 * C)], xbuf.at[ws2[c], pl.ds(0, 2 * C)], wsem.at[4 + c])
                     for c in range(2)]
        def w1_tile(kt, ct):
            c, j = divmod(ct, C // L)
            return xbuf[ws1[c // 2], (c % 2) * C + kt * L:(c % 2) * C + (kt + 1) * L, j * L:(j + 1) * L].astype(f32)
        def w2_tile(ct, j):
            c, r0 = divmod(ct * L, 2 * C)
            return xbuf[ws2[c], r0:r0 + L, j * L:(j + 1) * L].astype(f32)

        for cp in w1_copies:
            cp.start()
        for j in range(NX - 2):
            x_copy(j, (j + XO) % NX).start()
        zero[0] = 0
        acc[...] = jnp.zeros_like(acc)
        for buf, t in zip(mbs + a1b, mtail + (AR, AR)):
            buf[t:t + 24, :] = jnp.zeros((24, L), buf.dtype)
        row[0] = jnp.broadcast_to(dw_ref[...].astype(f32), (8, C))

        def ln_store(s, r0, lrow):
            o = xbuf[s, pl.ds(r0, LN), :].astype(f32) * jnp.concatenate([row[0]] * (LN // 8), axis=0)
            mu = jnp.sum(o, axis=-1, keepdims=True) * (1.0 / C)
            d = o - mu
            v = jnp.sum(d * d, axis=-1, keepdims=True)
            a = d * (lax.rsqrt(v + C * 1e-5) * (_A * C ** 0.5))
            for j in range(k1):
                lnbuf[j, pl.ds(lrow, LN), :] = a[:, j * L:(j + 1) * L]

        def ac_tile(lrow, dst, drow):
            halves = []
            for par in range(2):
                av = Lazy(m1 * k1, a1_steps, lambda v: lnbuf[v % k1, pl.ds(lrow + (v // k1) * 16 + par, 8, stride=2), :])
                halves.append([lincomb(a1_out[r], av)[0] for r in range(R1)])
            for r in range(R1):
                dst[pl.ds(drow + r * A1R, 8), :] = pack(halves[0][r], halves[1][r])

        def gelu_rows(getm, g, sq):
            mv = Lazy(K1, c1_steps, getm)
            res = []
            for e in range(m1 * n1):
                y, sg = lincomb(c1_out[e], mv)
                th = jnp.tanh(y * (y * y + _K0))
                hv = y * (th + 1.0) if sg > 0 else y * (th - 1.0)
                ct = (e % n1) * G1 + g
                sq[ct] = sq[ct] + hv * hv if ct in sq else hv * hv
                res.append(hv)
            return res

        def h_store(lo, hi, s, r0, g, dyn=0):
            for e in range(m1 * n1):
                hbuf[s, pl.ds(dyn + hrow((e % n1) * G1 + g, r0 + (e // n1) * (RB1 // 2)), 8), :] = pack(lo[e], hi[e])

        def flush_sq(sq):
            for ct in sorted(sq):
                acc[ct] += sq[ct]
            sq.clear()

        tpr = RB1 // ST
        ntick = len(dots1) // NM * tpr
        nt = RB1 // 8
        ge_at = [[] for _ in range(ntick)]
        for a in range(U1 * G1):
            ready = (max(z for z, d in enumerate(dots1) if d[0] == a) // NM + 1) * tpr
            for t in range(nt):
                z = max(((a + 1) * R1 * tpr) // NM + lag1 + (t * R1 * tpr) // (NM * nt), ready)
                if t % 2 and z >= ntick > zprev:
                    z = ntick - 1
                zprev = z
                ge_at[z % ntick].append((a, t, z >= ntick))
        carried = sorted({(a, t) for ev in ge_at for a, t, c in ev if c})
        per16 = m1 * (16 // LN)
        ln_at, ac_at = [[] for _ in range(ntick)], [[] for _ in range(ntick)]
        for u in range(U1):
            n_it = RB1 // 16 * per16
            for it in range(n_it):
                z = int((u + lnhi * it / n_it) * ntick / U1)
                ln_at[z].append((u + 1, it // per16, it % per16))
                if (it + 1) % per16 == 0:
                    ac_at[z + lnlag].append((u + 1, it // per16))

        def p1_body(s_prev, s_cur, sx_cur, sx_next, par):
            zp = pl.multiple_of(8 * par, 8)
            z0 = pl.multiple_of(zero[0], 8)
            sq, held, done, probes = {}, [], [], []
            for rho in range(len(dots1) // NM):
                res = []
                for a, r in dots1[rho * NM:(rho + 1) * NM]:
                    lhs = as_b(a1b[(a // G1) % 2][r * A1R:r * A1R + RB1 // 2, :])
                    res.append((a, r, jnp.dot(lhs, as_b(wbuf[(a % G1) * R1 + r]), preferred_element_type=f32)))
                for k in range(tpr):
                    pv = res[0][2][k * ST:k * ST + 8]
                    got = {(a, r): val[k * ST:(k + 1) * ST] for a, r, val in res}
                    for p, q, r, ca, cb in tris:
                        for a in sorted({a for a, r2 in got if r2 == r}):
                            m = got.pop((a, r))
                            got[a, p] = got[a, p] + m if ca > 0 else got[a, p] - m
                            got[a, q] = got[a, q] + m if cb > 0 else got[a, q] - m
                    for (a, r), val in got.items():
                        mbs[a % 4][pl.ds(z0 + kept1.index(r) * M1R + k * ST, ST), :] = val
                    if k % pmode == pmode - 1:
                        for a in sorted({a for a, _, _ in res}):
                            probes.append((len(done) + mdel, mbs[a % 4][mtail[a % 4] + 16:mtail[a % 4] + 24, :]))
                        probes.sort(key=lambda e: e[0])
                    for (pa, t, c) in ge_at[rho * tpr + k]:
                        pu, pg = divmod(pa, G1)
                        val = pv
                        if len(done) >= gd:
                            val = done[-gd] + pv
                            while probes and probes[0][0] <= len(done):
                                val = val + probes.pop(0)[1]
                        mbs[pa % 4][pl.ds(mtail[pa % 4] + zp, 8), :] = val
                        held.append(gelu_rows(lambda v: mbs[pa % 4][v * M1R + t * 8:v * M1R + (t + 1) * 8, :], pg, sq))
                        done.append(sum([sq[l * G1 + pg] for l in range(1, n1)], sq[pg]))
                        if len(held) == 2:
                            h_store(held[0], held[1], s_prev if c else s_cur, (pu * CM1 + (t - 1) * 8) // 2, pg)
                            held = []
                        if t == nt - 1:
                            flush_sq(sq)
                    for (nu, t, j) in ln_at[rho * tpr + k]:
                        q, j2 = divmod(j, 16 // LN)
                        ln_store(sx_cur if nu < U1 else sx_next, (nu % U1) * CM1 + q * RB1 + t * 16 + j2 * LN,
                                 z0 + (t % nln) * m1 * 16 + j * LN)
                    for (nu, t) in ac_at[rho * tpr + k]:
                        lnbuf[0, pl.ds(LR + zp, 8), :] = pv
                        ac_tile((t % nln) * m1 * 16, a1b[nu % 2], z0 + t * 8)
                        probes.append((len(done) + pdel, as_f(a1b[nu % 2][AR:AR + 8, :])))
            flush_sq(sq)

        for a in sorted({a % 4 for a, _ in carried}):
            mbs[a][0:K1 * M1R, :] = jnp.zeros((K1 * M1R, L), f32)
        for cp in w1_copies:
            cp.wait()
        for g in range(G1):
            for r in range(R1):
                val, sg = lincomb([(v, int(c) * sg1[r]) for v, c in enumerate(Vs1[r]) if c],
                                  lambda v: w1_tile(v // n1, (v % n1) * G1 + g))
                wbuf[g * R1 + r] = as_u((val if sg > 0 else -val).astype(bf16))

        for j in range(NX - 2, NX):
            x_copy(j, (j + XO) % NX).start()
        x_copy(0, XO).wait()

        def pro(t, _):
            for j in range(per16):
                q, j2 = divmod(j, 16 // LN)
                ln_store(XO, pl.multiple_of(t * 16, 16) + q * RB1 + j2 * LN, j * LN)
            ac_tile(0, a1e, pl.multiple_of(t * 8, 8))
        lax.fori_loop(0, RB1 // 16, pro, None)

        def p1(i, _):
            ip = jnp.maximum(i - 1, 0)

            @pl.when(i + 1 < T)
            def _():
                x_copy(i + 1, xslot(i + 1)).wait()

            @pl.when(tab_ref[2, i] >= 0)
            def _():
                hw_copy(tab_ref[2, i], tab_ref[0, i]).wait()
            p1_body(jnp.where(i > 0, tab_ref[0, ip], S - 1), tab_ref[0, i], xslot(i), xslot(jnp.minimum(i + 1, T - 1)),
                    lax.rem(i, 2))

            @pl.when(i + NX < T)
            def _():
                x_copy(i + NX, xslot(i)).start()

            @pl.when(i == T - NX + 1)
            def _():
                for cp in w2_copies:
                    cp.start()

            @pl.when(jnp.logical_and(i >= 1, tab_ref[1, ip] >= 0))
            def _():
                hw_copy(tab_ref[1, ip], tab_ref[0, ip]).start()
        lax.fori_loop(0, T, p1, None)
        for j in range(XA):
            x_copy(int(tab[3, j]), j).start()
        for a in sorted({a for a, _ in carried}):
            def epi(t, _):
                sq = {}
                r0 = pl.multiple_of(t * 16, 16)
                lo, hi = (gelu_rows(lambda v: mbs[a % 4][pl.ds(v * M1R + r0 + 8 * i, 8), :], a % G1, sq) for i in range(2))
                h_store(lo, hi, int(tab[0, T - 1]), (a // G1) * CM1 // 2, a % G1, pl.multiple_of(t * 8, 8))
                flush_sq(sq)
            lax.fori_loop(min(t for ca, t in carried if ca == a) // 2, nt // 2, epi, None)
        for cp in w2_copies:
            cp.wait()

        ss = jnp.concatenate([jnp.sum(acc[c], axis=0, keepdims=True) for c in range(NT)], axis=1) * (_GS * _GS)
        gx = jnp.sqrt(ss + 1e-6)
        nx = gx / (jnp.sum(gx, axis=-1, keepdims=True) * (1.0 / F) + 1e-6)
        sc = (g_ref[...].astype(f32).reshape(1, F) * nx + 1.0) * _GS
        sct = jnp.transpose(jnp.broadcast_to(sc, (L, F)))
        bt = jnp.transpose(jnp.broadcast_to(b_ref[...].astype(f32).reshape(1, F), (L, F)))
        for q in range(G2):
            for r in range(R2):
                def get(v):
                    ct = (v // n2) * G2 + q
                    return w2_tile(ct, v % n2) * sct[ct * L:(ct + 1) * L]
                val, sg = lincomb([(v, int(c) * sg2[r]) for v, c in enumerate(Vs2[r]) if c], get)
                wbuf[r * G2 + q] = as_u((val if sg > 0 else -val).astype(bf16))
        for j in range(n2):
            p = sum(w2_tile(ct, j) * bt[ct * L:(ct + 1) * L] for ct in range(NT))
            row[1, :, j * L:(j + 1) * L] = jnp.broadcast_to(jnp.sum(p, axis=0, keepdims=True), (8, L))
        sm1[0:R2 * M2R, :] = jnp.zeros((R2 * M2R, L), f32)

        def comb_tile(s, r0, q, dst, drow, dyn=0):
            raw = Lazy(m2 * k2, [], lambda v: hbuf[s, pl.ds(dyn + hrow((v % k2) * G2 + q, r0 + (v // k2) * (RB2 // 2)), 8), :])
            avs = [Lazy(m2 * k2, a2_steps, lambda v, i=i: unpack(raw(v), i)) for i in range(2)]
            for r in range(R2):
                dst[pl.ds(drow + (r * G2 + q) * A2R, 8), :] = as_f(
                    raw(a2_out[r][0][0]) if direct2[r] else pack(*(lincomb(a2_out[r], av)[0] for av in avs)))

        def out_tile(src, srow, sx, r0):
            mvs = [Lazy(R2, c2_steps, lambda v, i=i: src[pl.ds(srow + v * M2R + i, 8, stride=2), :]) for i in range(2)]
            for i in range(m2):
                rows = pl.ds(r0 + i * RB2, 16)
                xv = xbuf[sx, rows, :].astype(f32) + jnp.concatenate([row[1]] * 2, axis=0)
                res = []
                for l in range(n2):
                    ys = [lincomb(c2_out[i * n2 + l], mv) for mv in mvs]
                    y, z = jnp.concatenate([ys[0][0], ys[1][0]], axis=0), xv[:, l * L:(l + 1) * L]
                    res.append(z + y if ys[0][1] > 0 else z - y)
                xbuf[sx, rows, :] = jnp.concatenate(res, axis=1).astype(bf16)

        tp2 = RB2 // ST2
        ntick2 = U2 * R2 * tp2
        nt2 = RB2 // 16
        ot_at, cb_at = [[] for _ in range(ntick2)], [[] for _ in range(ntick2)]
        for u in range(U2):
            for t in range(nt2):
                z = (u + 1) * R2 * tp2 + lag2 + (t * (R2 * tp2 - lag2)) // nt2
                ot_at[z % ntick2].append((u, t, z >= ntick2))
            for k in range(G2 * nt2):
                cb_at[int((u + cbhi * k / (G2 * nt2)) * R2 * tp2)].append((u + 1, k % G2, k // G2))

        def p2_body(sx_prev, sx_cur, s_cur, s_next, par):
            z0 = pl.multiple_of(zero[0], 8)
            probes, ncb = [], 0
            for z in range(U2 * R2):
                u, r = divmod(z, R2)
                ys = [jnp.dot(as_b(a2b[u % 2][(r * G2 + q) * A2R:(r * G2 + q) * A2R + RB2 // 2, :]), as_b(wbuf[r * G2 + q]),
                              preferred_element_type=f32) for q in range(G2)]
                val = (ys[0] + ys[1]) + (ys[2] + ys[3])
                for k in range(tp2):
                    pv = val[k * ST2:k * ST2 + 8]
                    m2b[u % 2][pl.ds(z0 + r * M2R + k * ST2, ST2), :] = val[k * ST2:(k + 1) * ST2]
                    for (pu, t, c) in ot_at[z * tp2 + k]:
                        m2b[pu % 2][pl.ds(SR + pl.multiple_of(8 * par, 8), 8), :] = pv
                        xbuf[z0, TM:TM + 8, 0:L] = pv.astype(bf16)
                        out_tile(m2b[pu % 2], t * 16, sx_prev if c else sx_cur, pu * CM2 + t * 16)
                    for (nu, q, t) in cb_at[z * tp2 + k]:
                        pin = pv
                        while probes and probes[0][0] <= ncb:
                            pin = pin + probes.pop(0)[1]
                        hbuf[z0, HS:HS + 8, :] = as_u(pin)
                        comb_tile(s_cur if nu < U2 else s_next, ((nu % U2) * CM2 + t * 16) // 2, q, a2b[nu % 2], z0 + t * 8)
                        ncb += 1
                        probes.append((ncb + cd, a2b[nu % 2][BR + 8:BR + 16, :]))

        def pro2(t, _):
            r0 = pl.multiple_of(t * 8, 8)
            for q in range(G2):
                comb_tile(int(tab[4, 0]), 0, q, big0, r0, r0)
        lax.fori_loop(0, nt2, pro2, None)

        def p2(j, _):
            jn, jd, jp = jnp.minimum(j + 1, T - 1), jnp.minimum(j + D, T - 1), jnp.maximum(j - 1, 0)

            @pl.when(jnp.logical_and(j + 1 < T, tab_ref[5, jn] >= 0))
            def _():
                hr_head(tab_ref[5, jn], tab_ref[4, jn]).wait()

            @pl.when(tab_ref[5, j] >= 0)
            def _():
                hr_rest(tab_ref[5, j], tab_ref[4, j]).wait()
            x_copy(tab_ref[3, j], lax.rem(j, NX)).wait()
            p2_body(lax.rem(j + NX - 1, NX), lax.rem(j, NX), tab_ref[4, j], tab_ref[4, jn], lax.rem(j, 2))

            @pl.when(j >= 1)
            def _():
                o_copy(tab_ref[3, jp], lax.rem(jp, NX)).start()

            @pl.when(j + XA >= NX)
            def _():
                o_copy(tab_ref[3, jnp.maximum(j + XA - NX, 0)], lax.rem(j + XA, NX)).wait()

            @pl.when(j + XA < T)
            def _():
                x_copy(tab_ref[3, jnp.minimum(j + XA, T - 1)], lax.rem(j + XA, NX)).start()

            @pl.when(jnp.logical_and(j + D < T, tab_ref[5, jd] >= 0))
            def _():
                hr_head(tab_ref[5, jd], tab_ref[4, jd]).start()
                hr_rest(tab_ref[5, jd], tab_ref[4, jd]).start()
        lax.fori_loop(0, T, p2, None)

        def epi2(t, _):
            r0 = pl.multiple_of(t * 16, 16)
            out_tile(sm1, r0, (T - 1) % NX, (U2 - 1) * CM2 + r0)
        lax.fori_loop(0, nt2, epi2, None)
        o_copy(int(tab[3, T - 1]), (T - 1) % NX).start()
        for j in range(T + XA - NX, T):
            o_copy(int(tab[3, j]), j % NX).wait()

    vm = pl.BlockSpec(memory_space=pltpu.VMEM)
    hb = pl.BlockSpec(memory_space=pl.ANY)
    out, _ = pl.pallas_call(
        kernel,
        in_specs=[pl.BlockSpec(memory_space=pltpu.SMEM), hb, vm, hb, hb, vm, vm],
        out_specs=[hb, hb],
        out_shape=[jax.ShapeDtypeStruct((N, C), bf16), jax.ShapeDtypeStruct((nsp, HS, L), u32)],
        scratch_shapes=[
            pltpu.VMEM((NX, TM + 16, C), bf16), pltpu.VMEM((S, HS + 8, L), u32),
            pltpu.VMEM((max(G1 * R1, G2 * R2), L // 2, L), u32), pltpu.VMEM((NT, 8, L), f32), pltpu.VMEM((2, 8, C), f32),
            pltpu.SMEM((1,), jnp.int32), pltpu.VMEM((k1, LR + 16, L), f32),
            pltpu.VMEM((AR + 24, L), u32), pltpu.VMEM((AR + 24, L), u32),
            pltpu.VMEM((BR + 24, L), f32), pltpu.VMEM((BR + 24, L), f32),
            pltpu.VMEM((SR + 24, L), f32), pltpu.VMEM((SR + 24, L), f32),
            pltpu.SemaphoreType.DMA((NX,)), pltpu.SemaphoreType.DMA((2 * S,)), pltpu.SemaphoreType.DMA((NX,)),
            pltpu.SemaphoreType.DMA((6,)),
        ],
        compiler_params=pltpu.CompilerParams(vmem_limit_bytes=128 * 1024 * 1024),
    )(tab, x.reshape(N, C), dw.reshape(1, C), w1, w2, grn_g, grn_b)
    return out.reshape(B, H, W, C)
```

```python
import jax
import jax.numpy as jnp
import numpy as np
from jax import lax
import jax.experimental.pallas as pl
import jax.experimental.pallas.tpu as pltpu

L = 128
NM = 4

_C0 = float(np.sqrt(2.0 / np.pi))
_C1 = _C0 * 0.044715
_A = _C1 ** (1.0 / 3.0)
_K0 = _C0 / _A
_GS = 0.5 / _A


def _scheme(shape, products):
    m, k, n = shape
    U, V, W = (np.array([p[i] for p in products]) for i in range(3))
    want = np.zeros((m * k, k * n, m * n), int)
    for i in range(m):
        for j in range(k):
            for l in range(n):
                want[i * k + j, j * n + l, i * n + l] = 1
    assert (np.einsum("ra,rb,rc->abc", U, V, W) == want).all()
    return shape, U, V, W


SCHEME1 = _scheme((2, 3, 3), [
    ([0, 0, 0, 0, 0, -1], [0, 0, 0, -1, 0, 0, -1, 1, 0], [-1, 0, 0, 1, 0, 0]),
    ([-1, -1, 0, -1, -1, 0], [0, 0, 1, 1, 0, 0, 0, 0, 0], [0, 0, 0, 0, 0, -1]),
    ([1, 0, 1, 0, 0, 0], [0, 0, 0, 0, 0, 0, 0, -1, 0], [-1, -1, 0, 1, 1, 0]),
    ([1, 0, 0, 0, 0, 0], [0, 1, -1, 0, -1, 1, 0, -1, 0], [0, 1, 0, 0, 0, 0]),
    ([0, 0, 0, 0, 1, 0], [0, 0, 0, 0, -1, 0, 0, 0, 0], [0, 1, 1, 0, -1, -1]),
    ([-1, -1, 0, 0, 0, -1], [0, 0, 0, -1, 0, 0, 0, 0, 1], [1, 0, 0, 0, 0, -1]),
    ([1, 1, 0, 0, 1, 0], [0, 0, -1, 0, -1, 1, 0, 0, 0], [0, -1, -1, 0, 0, 1]),
    ([0, 0, 0, -1, 0, 0], [-1, 1, 0, 1, 0, 0, 0, 0, 0], [0, 0, 0, 0, -1, 0]),
    ([0, 0, -1, 0, 0, -1], [-1, 0, 0, 1, 0, 0, 1, 0, 1], [-1, 0, 0, 0, 0, 0]),
    ([0, 1, 0, 0, 1, 0], [0, 0, 1, 0, 0, -1, 0, 0, 0], [0, -1, -1, 0, 0, 0]),
    ([-1, 0, -1, 0, 0, -1], [1, 0, 0, -1, 0, 0, 0, -1, 0], [-1, 0, 0, 1, 1, 0]),
    ([-1, -1, 1, 0, 0, 0], [0, 0, 0, 0, 0, 0, 0, 0, -1], [1, 0, -1, 0, 0, 0]),
    ([-1, 0, -1, -1, 0, -1], [-1, 0, 0, 1, 0, 0, 0, 0, 0], [0, 0, 0, 1, 1, 0]),
    ([0, 0, 0, 1, 1, -1], [0, 0, 0, 1, 0, 0, 0, 0, 0], [0, 0, 0, 1, 0, -1]),
    ([-1, -1, 0, 0, 0, 0], [0, 0, 0, 0, -1, 1, 0, 0, 1], [0, 0, -1, 0, 0, 1]),
])
SCHEME2 = _scheme((2, 3, 3), [
    ([0, 0, 0, 0, 0, 1], [1, 0, 1, 0, 0, 0, -1, 0, 0], [-1, 0, 0, -1, 0, 0]),
    ([1, 0, 0, -1, 1, 0], [0, 0, -1, 0, -1, 0, 0, 0, 0], [1, -1, -1, 0, -1, 0]),
    ([0, -1, -1, 0, 0, 1], [0, 0, 0, -1, 0, -1, 0, 0, 1], [1, 0, 0, 0, 0, 1]),
    ([1, 0, 1, 0, 0, 0], [0, 0, 0, 0, 0, 0, 0, -1, 0], [-1, -1, 0, 0, 0, 0]),
    ([0, 0, 0, -1, 0, -1], [-1, 0, -1, 0, 0, 0, 0, 0, 0], [0, 0, 0, 1, 1, 0]),
    ([-1, 0, 0, 0, 0, -1], [1, 0, 1, 0, 0, 0, 0, -1, 0], [-1, 0, 0, 0, 1, 0]),
    ([0, 1, 0, 0, 0, 0], [0, 0, 0, 0, -1, 1, 0, 0, -1], [-1, 0, 1, 0, 0, 0]),
    ([0, 0, 1, 0, 0, -1], [0, 0, 0, -1, 0, -1, 1, -1, 1], [1, 0, 0, 0, 0, 0]),
    ([-1, 0, 0, 0, 0, 0], [0, 1, -1, 0, 0, 0, 0, -1, 0], [0, -1, 0, 0, -1, 0]),
    ([0, -1, -1, 0, 1, 1], [0, 0, 0, 1, 0, 1, 0, 0, 0], [0, 0, 0, 0, 0, 1]),
    ([0, 0, 0, 0, 1, 0], [0, 0, -1, 1, 0, 0, 0, 0, 0], [0, 0, 0, 1, 0, -1]),
    ([-1, 1, 0, 1, -1, 0], [0, 0, 0, 0, 1, 0, 0, 0, 0], [-1, 1, 1, 0, 0, 0]),
    ([0, 0, 0, 1, -1, 0], [0, 0, 1, 0, 0, 0, 0, 0, 0], [-1, 1, 1, -1, 1, 1]),
    ([0, -1, -1, 0, 0, 0], [0, 0, 0, 0, 0, 0, 0, 0, -1], [0, 0, 1, 0, 0, 1]),
    ([1, 0, 0, -1, 0, 0], [-1, 1, -1, 0, 1, 0, 0, 0, 0], [0, 0, 0, 0, -1, 0]),
])


def cse(rows):
    R = [list(map(int, r)) for r in rows]; steps = []
    while True:
        n = len(R[0]); best = 1; arg = None
        for i in range(n):
            for j in range(i+1, n):
                a = sum(1 for r in R if r[i]*r[j] > 0); b = sum(1 for r in R if r[i]*r[j] < 0)
                if a > best: best = a; arg = (i, j, 1)
                if b > best: best = b; arg = (i, j, -1)
        if arg is None: break
        i, j, s = arg; steps.append(arg)
        for r in R:
            if r[i]*r[j] == s: r.append(r[i]); r[i] = 0; r[j] = 0
            else: r.append(0)
    return steps, [[(v, c) for v, c in enumerate(r) if c] for r in R]


def lincomb(terms, get):
    pos = [v for v, c in terms if c > 0]
    neg = [v for v, c in terms if c < 0]
    sign = 1
    if not pos:
        pos, neg, sign = neg, [], -1
    acc = get(pos[0])
    for v, c in terms:
        if v == pos[0]:
            continue
        acc = acc + get(v) if c * sign > 0 else acc - get(v)
    return acc, sign


class Lazy:
    def __init__(self, nin, steps, leaf):
        self.nin, self.steps, self.leaf, self.memo = nin, steps, leaf, {}
    def __call__(self, v):
        if v not in self.memo:
            if v < self.nin:
                self.memo[v] = self.leaf(v)
            else:
                i, j, s = self.steps[v - self.nin]
                self.memo[v] = self(i) + self(j) if s > 0 else self(i) - self(j)
        return self.memo[v]


def schedule(T, S, NS, D):
    spread = S - NS
    keep = [((i + 1) * spread) // (T - NS) > (i * spread) // (T - NS) for i in range(T - NS)] + [True] * NS
    slot1, spill, wait1, last, nxt, rr, nsp = [], [], [], {}, NS, 0, 0
    for i in range(T):
        if keep[i] and i < T - NS:
            slot1.append(nxt); wait1.append(-1); nxt += 1
        else:
            slot1.append(rr); wait1.append(last.get(rr, -1)); last[rr] = i; rr = (rr + 1) % NS
        spill.append(-1 if keep[i] else nsp)
        nsp += not keep[i]
    kept = [i for i in range(T) if keep[i]][::-1]
    rest = [i for i in range(T) if not keep[i]]
    order, nk = kept[:D], len(kept) - D
    kept = kept[D:]
    for j in range(T - D):
        order.append(kept.pop(0) if ((j + 1) * nk) // (T - D) > (j * nk) // (T - D) else rest.pop(0))
    slot2 = []
    for j, i in enumerate(order):
        slot2.append(slot1[i] if keep[i] else slot2[j - D])
    src2 = [spill[i] for i in order]
    wsp = [spill[w] if w >= 0 else -1 for w in wait1]
    return np.array([slot1, spill, wsp, order, slot2, src2], np.int32), nsp


def fold_triangles(W):
    R = len(W)
    tri = [(p, q, r, a, b) for p in range(R) for q in range(p + 1, R) for r in range(R) for a in (1, -1) for b in (1, -1)
           if r != p and r != q and (W[r] == a * W[p] + b * W[q]).all()]
    def cost(sel):
        keep = [i for i in range(R) if i not in [t[2] for t in sel]]
        steps, outs = cse(W[keep].T)
        return 2 * len(sel) + len(steps) + sum(len(t) - 1 for t in outs)
    level, best = [()], ()
    while level:
        best = min(level, key=cost)
        level = [sel + (t,) for sel in level for t in tri
                 if (not sel or t > sel[-1]) and not set(t[:3]) & set(i for u in sel for i in u[:3])]
    return best


RB1 = 128
U1 = 4
TP = 2
RB2 = 64
U2 = 8
NX = 5
XA = 3
S = 38
NS = 5
D = 3
ST = 16
lag1 = 8
gd = 3
lnhi = 0.85
lnlag = 4
nln = 4
pmode = 4
mdel = 4
pdel = 1
LN = 8
ST2 = 32
lag2 = 1
cbhi = 0.8
cd = 2


@jax.jit
def pallas_standalone__modern_conv_block_slak__vision_kernel(x, dw, w1, w2, grn_g, grn_b):
    B, H, W, C = x.shape
    assert B == 1 and dw.shape[:2] == (1, 1)
    F = w1.shape[1]
    N = B * H * W
    f32, bf16, u32 = jnp.float32, jnp.bfloat16, jnp.uint32
    (m1, k1, n1), Us1, Vs1, Ws1 = SCHEME1
    (m2, k2, n2), Us2, Vs2, Ws2 = SCHEME2
    R1, R2 = len(Us1), len(Us2)
    assert k1 * L == C and n2 * L == C
    G1, G2 = F // (n1 * L), F // (k2 * L)
    a1_steps, a1_out = cse(Us1)
    tris = fold_triangles(Ws1)
    kept1 = [r for r in range(R1) if r not in [t[2] for t in tris]]
    K1 = len(kept1)
    c1_steps, c1_out = cse(Ws1[kept1].T)
    loose = [r for r in range(R1) if r not in [i for t in tris for i in t[:3]]]
    UU = U1 * TP
    dots1, pend = [], [(list(tris), [(a, r) for r in loose]) for a in range(UU * G1)]
    for a in range(UU * G1):
        todo, free = pend[a]
        while todo or free:
            if todo and len(dots1) % NM <= 1 and (len(dots1) % NM == 1 or len(free) <= len(todo) or len(tris) < 4):
                dots1 += [(a, r) for r in todo.pop(0)[:3]]
            else:
                dots1.append((free or pend[a + 1][1]).pop(0))
    a2_steps, a2_out = cse(Us2)
    c2_steps, c2_out = cse(Ws2.T)
    sg1 = [1 if any(c > 0 for _, c in t) else -1 for t in a1_out]
    sg2 = [1 if any(c > 0 for _, c in t) else -1 for t in a2_out]
    direct2 = [len(t) == 1 and t[0][0] < m2 * k2 for t in a2_out]
    CM1, CM2 = m1 * RB1, m2 * RB2
    TM = CM1 * U1
    assert TM == CM2 * U2 and N % TM == 0 and U1 % 2 == 0 and U2 % 2 == 0 and (U1 * G1) % 4 == 0
    assert (CM2 // 2) % (RB1 // 2) == 0
    T, NT = N // TM, F // L
    tab, nsp = schedule(T, S, NS, D)
    assert T % TP == 0 and NS >= 2 * TP + 1
    M1R, A1R, M2R, A2R = RB1 + 8, RB1 // 2 + 8, RB2 + 8, RB2 // 2 + 8
    HC = CM2 // 2
    HS = NT * TM // 2
    hrow = lambda ct, r: (r // HC) * (NT * HC) + ct * HC + r % HC
    BR = max(K1 * M1R, R2 * G2 * A2R)
    SR = max(K1 * M1R, R2 * M2R)
    AR = R1 * A1R
    LR = nln * m1 * 16
    pack = lambda lo, hi: pltpu.pack_elementwise([lo, hi], packed_dtype=bf16)
    unpack = lambda w, i: pltpu.unpack_elementwise(w, index=i, packed_dtype=bf16, unpacked_dtype=f32)
    as_u, as_f, as_b = (lambda v: pltpu.bitcast(v, u32)), (lambda v: pltpu.bitcast(v, f32)), (lambda v: pltpu.bitcast(v, bf16))

    def kernel(tab_ref, x_hbm, dw_ref, w1_hbm, w2_hbm, g_ref, b_ref, o_hbm, h_hbm,
               xbuf, hbuf, wbuf, acc, row, zero, lnbuf, a1e, a1o, big0, big1, sm0, sm1, xsem, hsem, osem, wsem):
        a1b, mbs, a2b, m2b = (a1e, a1o), (big0, big1, sm0, sm1), (big0, big1), (sm0, sm1)
        mtail = (BR, BR, SR, SR)

        mk = pltpu.make_async_copy
        def x_copy(i, s): return mk(x_hbm.at[pl.ds(i * TM, TM)], xbuf.at[s, pl.ds(0, TM)], xsem.at[s])
        def hw_copy(i, s): return mk(hbuf.at[s, pl.ds(0, HS)], h_hbm.at[i], hsem.at[s])
        def hr_head(i, s): return mk(h_hbm.at[i, pl.ds(0, NT * HC)], hbuf.at[s, pl.ds(0, NT * HC)], hsem.at[s])
        def hr_rest(i, s): return mk(h_hbm.at[i, pl.ds(NT * HC, HS - NT * HC)], hbuf.at[s, pl.ds(NT * HC, HS - NT * HC)], hsem.at[S + s])
        def o_copy(i, s): return mk(xbuf.at[s, pl.ds(0, TM)], o_hbm.at[pl.ds(i * TM, TM)], osem.at[s])

        XO = (XA - (T - NX)) % NX
        xslot = lambda i: lax.rem(i + XO, NX)
        ws1, ws2 = [(NX - 2 + c + XO) % NX for c in range(2)], [XA, XA + 1]
        w1_copies = [pltpu.make_async_copy(w1_hbm.at[:, pl.ds(c * C, C)], xbuf.at[ws1[c // 2], pl.ds((c % 2) * C, C)], wsem.at[c])
                     for c in range(4)]
        w2_copies = [pltpu.make_async_copy(w2_hbm.at[pl.ds(c * 2 * C, 2 * C)], xbuf.at[ws2[c], pl.ds(0, 2 * C)], wsem.at[4 + c])
                     for c in range(2)]
        def w1_tile(kt, ct):
            c, j = divmod(ct, C // L)
            return xbuf[ws1[c // 2], (c % 2) * C + kt * L:(c % 2) * C + (kt + 1) * L, j * L:(j + 1) * L].astype(f32)
        def w2_tile(ct, j):
            c, r0 = divmod(ct * L, 2 * C)
            return xbuf[ws2[c], r0:r0 + L, j * L:(j + 1) * L].astype(f32)

        for cp in w1_copies:
            cp.start()
        for j in range(NX - 2):
            x_copy(j, (j + XO) % NX).start()
        zero[0] = 0
        acc[...] = jnp.zeros_like(acc)
        for buf, t in zip(mbs + a1b, mtail + (AR, AR)):
            buf[t:t + 24, :] = jnp.zeros((24, L), buf.dtype)
        row[0] = jnp.broadcast_to(dw_ref[...].astype(f32), (8, C))

        def ln_store(s, r0, lrow):
            o = xbuf[s, pl.ds(r0, LN), :].astype(f32) * jnp.concatenate([row[0]] * (LN // 8), axis=0)
            mu = jnp.sum(o, axis=-1, keepdims=True) * (1.0 / C)
            d = o - mu
            v = jnp.sum(d * d, axis=-1, keepdims=True)
            a = d * (lax.rsqrt(v + C * 1e-5) * (_A * C ** 0.5))
            for j in range(k1):
                lnbuf[j, pl.ds(lrow, LN), :] = a[:, j * L:(j + 1) * L]

        def ac_tile(lrow, dst, drow):
            halves = []
            for par in range(2):
                av = Lazy(m1 * k1, a1_steps, lambda v: lnbuf[v % k1, pl.ds(lrow + (v // k1) * 16 + par, 8, stride=2), :])
                halves.append([lincomb(a1_out[r], av)[0] for r in range(R1)])
            for r in range(R1):
                dst[pl.ds(drow + r * A1R, 8), :] = pack(halves[0][r], halves[1][r])

        def gelu_rows(getm, g, sq):
            mv = Lazy(K1, c1_steps, getm)
            res = []
            for e in range(m1 * n1):
                y, sg = lincomb(c1_out[e], mv)
                th = jnp.tanh(y * (y * y + _K0))
                hv = y * (th + 1.0) if sg > 0 else y * (th - 1.0)
                ct = (e % n1) * G1 + g
                sq[ct] = sq[ct] + hv * hv if ct in sq else hv * hv
                res.append(hv)
            return res

        def h_store(lo, hi, s, r0, g, dyn=0):
            for e in range(m1 * n1):
                hbuf[s, pl.ds(dyn + hrow((e % n1) * G1 + g, r0 + (e // n1) * (RB1 // 2)), 8), :] = pack(lo[e], hi[e])

        def flush_sq(sq):
            for ct in sorted(sq):
                acc[ct] += sq[ct]
            sq.clear()

        tpr = RB1 // ST
        ntick = len(dots1) // NM * tpr
        nt = RB1 // 8
        ge_at = [[] for _ in range(ntick)]
        for a in range(UU * G1):
            ready = (max(z for z, d in enumerate(dots1) if d[0] == a) // NM + 1) * tpr
            for t in range(nt):
                z = max(((a + 1) * R1 * tpr) // NM + lag1 + (t * R1 * tpr) // (NM * nt), ready)
                if t % 2 and z >= ntick > zprev:
                    z = ntick - 1
                zprev = z
                ge_at[z % ntick].append((a, t, z >= ntick))
        carried = sorted({(a, t) for ev in ge_at for a, t, c in ev if c})
        per16 = m1 * (16 // LN)
        ln_at, ac_at = [[] for _ in range(ntick)], [[] for _ in range(ntick)]
        for u in range(UU):
            n_it = RB1 // 16 * per16
            for it in range(n_it):
                z = int((u + lnhi * it / n_it) * ntick / UU)
                ln_at[z].append((u + 1, it // per16, it % per16))
                if (it + 1) % per16 == 0:
                    ac_at[z + lnlag].append((u + 1, it // per16))

        def p1_body(hs, xs, par):
            zp = pl.multiple_of(8 * par, 8)
            z0 = pl.multiple_of(zero[0], 8)
            sq, held, done, probes = {}, [], [], []
            for rho in range(len(dots1) // NM):
                res = []
                for a, r in dots1[rho * NM:(rho + 1) * NM]:
                    lhs = as_b(a1b[(a // G1) % 2][r * A1R:r * A1R + RB1 // 2, :])
                    res.append((a, r, jnp.dot(lhs, as_b(wbuf[(a % G1) * R1 + r]), preferred_element_type=f32)))
                for k in range(tpr):
                    pv = res[0][2][k * ST:k * ST + 8]
                    got = {(a, r): val[k * ST:(k + 1) * ST] for a, r, val in res}
                    for p, q, r, ca, cb in tris:
                        for a in sorted({a for a, r2 in got if r2 == r}):
                            m = got.pop((a, r))
                            got[a, p] = got[a, p] + m if ca > 0 else got[a, p] - m
                            got[a, q] = got[a, q] + m if cb > 0 else got[a, q] - m
                    for (a, r), val in got.items():
                        mbs[a % 4][pl.ds(z0 + kept1.index(r) * M1R + k * ST, ST), :] = val
                    if k % pmode == pmode - 1:
                        for a in sorted({a for a, _, _ in res}):
                            probes.append((len(done) + mdel, mbs[a % 4][mtail[a % 4] + 16:mtail[a % 4] + 24, :]))
                        probes.sort(key=lambda e: e[0])
                    for (pa, t, c) in ge_at[rho * tpr + k]:
                        pu, pg = divmod(pa, G1)
                        val = pv
                        if len(done) >= gd:
                            val = done[-gd] + pv
                            while probes and probes[0][0] <= len(done):
                                val = val + probes.pop(0)[1]
                        mbs[pa % 4][pl.ds(mtail[pa % 4] + zp, 8), :] = val
                        held.append(gelu_rows(lambda v: mbs[pa % 4][v * M1R + t * 8:v * M1R + (t + 1) * 8, :], pg, sq))
                        done.append(sum([sq[l * G1 + pg] for l in range(1, n1)], sq[pg]))
                        if len(held) == 2:
                            h_store(held[0], held[1], hs[0 if c else 1 + pu // U1], ((pu % U1) * CM1 + (t - 1) * 8) // 2, pg)
                            held = []
                        if t == nt - 1:
                            flush_sq(sq)
                    for (nu, t, j) in ln_at[rho * tpr + k]:
                        q, j2 = divmod(j, 16 // LN)
                        ln_store(xs[nu // U1], (nu % U1) * CM1 + q * RB1 + t * 16 + j2 * LN,
                                 z0 + (t % nln) * m1 * 16 + j * LN)
                    for (nu, t) in ac_at[rho * tpr + k]:
                        lnbuf[0, pl.ds(LR + zp, 8), :] = pv
                        ac_tile((t % nln) * m1 * 16, a1b[nu % 2], z0 + t * 8)
                        probes.append((len(done) + pdel, as_f(a1b[nu % 2][AR:AR + 8, :])))
            flush_sq(sq)

        for a in sorted({a % 4 for a, _ in carried}):
            mbs[a][0:K1 * M1R, :] = jnp.zeros((K1 * M1R, L), f32)
        for cp in w1_copies:
            cp.wait()
        for g in range(G1):
            for r in range(R1):
                val, sg = lincomb([(v, int(c) * sg1[r]) for v, c in enumerate(Vs1[r]) if c],
                                  lambda v: w1_tile(v // n1, (v % n1) * G1 + g))
                wbuf[g * R1 + r] = as_u((val if sg > 0 else -val).astype(bf16))

        for j in range(NX - 2, NX):
            x_copy(j, (j + XO) % NX).start()
        x_copy(0, XO).wait()

        def pro(t, _):
            for j in range(per16):
                q, j2 = divmod(j, 16 // LN)
                ln_store(XO, pl.multiple_of(t * 16, 16) + q * RB1 + j2 * LN, j * LN)
            ac_tile(0, a1e, pl.multiple_of(t * 8, 8))
        lax.fori_loop(0, RB1 // 16, pro, None)

        def p1(it, _):
            i = it * TP
            for d in range(TP):
                @pl.when(i + d + 1 < T)
                def _():
                    x_copy(i + d + 1, xslot(i + d + 1)).wait()

                @pl.when(tab_ref[2, i + d] >= 0)
                def _():
                    hw_copy(tab_ref[2, i + d], tab_ref[0, i + d]).wait()
            p1_body([jnp.where(i > 0, tab_ref[0, jnp.maximum(i - 1, 0)], S - 1)] + [tab_ref[0, i + d] for d in range(TP)],
                    [xslot(jnp.minimum(i + d, T - 1)) for d in range(TP + 1)], lax.rem(it, 2))
            for d in range(TP):
                @pl.when(i + d + NX < T)
                def _():
                    x_copy(i + d + NX, xslot(i + d)).start()

            @pl.when(it == (T - NX + 1) // TP)
            def _():
                for cp in w2_copies:
                    cp.start()
            for d in range(TP):
                ip = jnp.maximum(i + d - 1, 0)

                @pl.when(jnp.logical_and(i + d >= 1, tab_ref[1, ip] >= 0))
                def _():
                    hw_copy(tab_ref[1, ip], tab_ref[0, ip]).start()
        lax.fori_loop(0, T // TP, p1, None)
        for j in range(XA):
            x_copy(int(tab[3, j]), j).start()
        for a in sorted({a for a, _ in carried}):
            def epi(t, _):
                sq = {}
                r0 = pl.multiple_of(t * 16, 16)
                lo, hi = (gelu_rows(lambda v: mbs[a % 4][pl.ds(v * M1R + r0 + 8 * i, 8), :], a % G1, sq) for i in range(2))
                h_store(lo, hi, int(tab[0, T - 1]), ((a // G1) % U1) * CM1 // 2, a % G1, pl.multiple_of(t * 8, 8))
                flush_sq(sq)
            lax.fori_loop(min(t for ca, t in carried if ca == a) // 2, nt // 2, epi, None)
        for cp in w2_copies:
            cp.wait()

        ss = jnp.concatenate([jnp.sum(acc[c], axis=0, keepdims=True) for c in range(NT)], axis=1) * (_GS * _GS)
        gx = jnp.sqrt(ss + 1e-6)
        nx = gx / (jnp.sum(gx, axis=-1, keepdims=True) * (1.0 / F) + 1e-6)
        sc = (g_ref[...].astype(f32).reshape(1, F) * nx + 1.0) * _GS
        sct = jnp.transpose(jnp.broadcast_to(sc, (L, F)))
        bt = jnp.transpose(jnp.broadcast_to(b_ref[...].astype(f32).reshape(1, F), (L, F)))
        for q in range(G2):
            for r in range(R2):
                def get(v):
                    ct = (v // n2) * G2 + q
                    return w2_tile(ct, v % n2) * sct[ct * L:(ct + 1) * L]
                val, sg = lincomb([(v, int(c) * sg2[r]) for v, c in enumerate(Vs2[r]) if c], get)
                wbuf[r * G2 + q] = as_u((val if sg > 0 else -val).astype(bf16))
        for j in range(n2):
            p = sum(w2_tile(ct, j) * bt[ct * L:(ct + 1) * L] for ct in range(NT))
            row[1, :, j * L:(j + 1) * L] = jnp.broadcast_to(jnp.sum(p, axis=0, keepdims=True), (8, L))
        sm1[0:R2 * M2R, :] = jnp.zeros((R2 * M2R, L), f32)

        def comb_tile(s, r0, q, dst, drow, dyn=0):
            raw = Lazy(m2 * k2, [], lambda v: hbuf[s, pl.ds(dyn + hrow((v % k2) * G2 + q, r0 + (v // k2) * (RB2 // 2)), 8), :])
            avs = [Lazy(m2 * k2, a2_steps, lambda v, i=i: unpack(raw(v), i)) for i in range(2)]
            for r in range(R2):
                dst[pl.ds(drow + (r * G2 + q) * A2R, 8), :] = as_f(
                    raw(a2_out[r][0][0]) if direct2[r] else pack(*(lincomb(a2_out[r], av)[0] for av in avs)))

        def out_tile(src, srow, sx, r0):
            mvs = [Lazy(R2, c2_steps, lambda v, i=i: src[pl.ds(srow + v * M2R + i, 8, stride=2), :]) for i in range(2)]
            for i in range(m2):
                rows = pl.ds(r0 + i * RB2, 16)
                xv = xbuf[sx, rows, :].astype(f32) + jnp.concatenate([row[1]] * 2, axis=0)
                res = []
                for l in range(n2):
                    ys = [lincomb(c2_out[i * n2 + l], mv) for mv in mvs]
                    y, z = jnp.concatenate([ys[0][0], ys[1][0]], axis=0), xv[:, l * L:(l + 1) * L]
                    res.append(z + y if ys[0][1] > 0 else z - y)
                xbuf[sx, rows, :] = jnp.concatenate(res, axis=1).astype(bf16)

        tp2 = RB2 // ST2
        ntick2 = U2 * R2 * tp2
        nt2 = RB2 // 16
        ot_at, cb_at = [[] for _ in range(ntick2)], [[] for _ in range(ntick2)]
        for u in range(U2):
            for t in range(nt2):
                z = (u + 1) * R2 * tp2 + lag2 + (t * (R2 * tp2 - lag2)) // nt2
                ot_at[z % ntick2].append((u, t, z >= ntick2))
            for k in range(G2 * nt2):
                cb_at[int((u + cbhi * k / (G2 * nt2)) * R2 * tp2)].append((u + 1, k % G2, k // G2))

        def p2_body(sx_prev, sx_cur, s_cur, s_next, par):
            z0 = pl.multiple_of(zero[0], 8)
            probes, ncb = [], 0
            for z in range(U2 * R2):
                u, r = divmod(z, R2)
                ys = [jnp.dot(as_b(a2b[u % 2][(r * G2 + q) * A2R:(r * G2 + q) * A2R + RB2 // 2, :]), as_b(wbuf[r * G2 + q]),
                              preferred_element_type=f32) for q in range(G2)]
                val = (ys[0] + ys[1]) + (ys[2] + ys[3])
                for k in range(tp2):
                    pv = val[k * ST2:k * ST2 + 8]
                    m2b[u % 2][pl.ds(z0 + r * M2R + k * ST2, ST2), :] = val[k * ST2:(k + 1) * ST2]
                    for (pu, t, c) in ot_at[z * tp2 + k]:
                        m2b[pu % 2][pl.ds(SR + pl.multiple_of(8 * par, 8), 8), :] = pv
                        xbuf[z0, TM:TM + 8, 0:L] = pv.astype(bf16)
                        out_tile(m2b[pu % 2], t * 16, sx_prev if c else sx_cur, pu * CM2 + t * 16)
                    for (nu, q, t) in cb_at[z * tp2 + k]:
                        pin = pv
                        while probes and probes[0][0] <= ncb:
                            pin = pin + probes.pop(0)[1]
                        hbuf[z0, HS:HS + 8, :] = as_u(pin)
                        comb_tile(s_cur if nu < U2 else s_next, ((nu % U2) * CM2 + t * 16) // 2, q, a2b[nu % 2], z0 + t * 8)
                        ncb += 1
                        probes.append((ncb + cd, a2b[nu % 2][BR + 8:BR + 16, :]))

        def pro2(t, _):
            r0 = pl.multiple_of(t * 8, 8)
            for q in range(G2):
                comb_tile(int(tab[4, 0]), 0, q, big0, r0, r0)
        lax.fori_loop(0, nt2, pro2, None)

        def p2(j, _):
            jn, jd, jp = jnp.minimum(j + 1, T - 1), jnp.minimum(j + D, T - 1), jnp.maximum(j - 1, 0)

            @pl.when(jnp.logical_and(j + 1 < T, tab_ref[5, jn] >= 0))
            def _():
                hr_head(tab_ref[5, jn], tab_ref[4, jn]).wait()

            @pl.when(tab_ref[5, j] >= 0)
            def _():
                hr_rest(tab_ref[5, j], tab_ref[4, j]).wait()
            x_copy(tab_ref[3, j], lax.rem(j, NX)).wait()
            p2_body(lax.rem(j + NX - 1, NX), lax.rem(j, NX), tab_ref[4, j], tab_ref[4, jn], lax.rem(j, 2))

            @pl.when(j >= 1)
            def _():
                o_copy(tab_ref[3, jp], lax.rem(jp, NX)).start()

            @pl.when(j + XA >= NX)
            def _():
                o_copy(tab_ref[3, jnp.maximum(j + XA - NX, 0)], lax.rem(j + XA, NX)).wait()

            @pl.when(j + XA < T)
            def _():
                x_copy(tab_ref[3, jnp.minimum(j + XA, T - 1)], lax.rem(j + XA, NX)).start()

            @pl.when(jnp.logical_and(j + D < T, tab_ref[5, jd] >= 0))
            def _():
                hr_head(tab_ref[5, jd], tab_ref[4, jd]).start()
                hr_rest(tab_ref[5, jd], tab_ref[4, jd]).start()
        lax.fori_loop(0, T, p2, None)

        def epi2(t, _):
            r0 = pl.multiple_of(t * 16, 16)
            out_tile(sm1, r0, (T - 1) % NX, (U2 - 1) * CM2 + r0)
        lax.fori_loop(0, nt2, epi2, None)
        o_copy(int(tab[3, T - 1]), (T - 1) % NX).start()
        for j in range(T + XA - NX, T):
            o_copy(int(tab[3, j]), j % NX).wait()

    vm = pl.BlockSpec(memory_space=pltpu.VMEM)
    hb = pl.BlockSpec(memory_space=pl.ANY)
    out, _ = pl.pallas_call(
        kernel,
        in_specs=[pl.BlockSpec(memory_space=pltpu.SMEM), hb, vm, hb, hb, vm, vm],
        out_specs=[hb, hb],
        out_shape=[jax.ShapeDtypeStruct((N, C), bf16), jax.ShapeDtypeStruct((nsp, HS, L), u32)],
        scratch_shapes=[
            pltpu.VMEM((NX, TM + 16, C), bf16), pltpu.VMEM((S, HS + 8, L), u32),
            pltpu.VMEM((max(G1 * R1, G2 * R2), L // 2, L), u32), pltpu.VMEM((NT, 8, L), f32), pltpu.VMEM((2, 8, C), f32),
            pltpu.SMEM((1,), jnp.int32), pltpu.VMEM((k1, LR + 16, L), f32),
            pltpu.VMEM((AR + 24, L), u32), pltpu.VMEM((AR + 24, L), u32),
            pltpu.VMEM((BR + 24, L), f32), pltpu.VMEM((BR + 24, L), f32),
            pltpu.VMEM((SR + 24, L), f32), pltpu.VMEM((SR + 24, L), f32),
            pltpu.SemaphoreType.DMA((NX,)), pltpu.SemaphoreType.DMA((2 * S,)), pltpu.SemaphoreType.DMA((NX,)),
            pltpu.SemaphoreType.DMA((6,)),
        ],
        compiler_params=pltpu.CompilerParams(vmem_limit_bytes=128 * 1024 * 1024, disable_bounds_checks=True),
    )(tab, x.reshape(N, C), dw.reshape(1, C), w1, w2, grn_g, grn_b)
    return out.reshape(B, H, W, C)
```

```python
import jax
import jax.numpy as jnp
import numpy as np
from jax import lax
import jax.experimental.pallas as pl
import jax.experimental.pallas.tpu as pltpu

L = 128
NM = 4

_C0 = float(np.sqrt(2.0 / np.pi))
_C1 = _C0 * 0.044715
_A = _C1 ** (1.0 / 3.0)
_K0 = _C0 / _A
_GS = 0.5 / _A


def _scheme(shape, products):
    m, k, n = shape
    U, V, W = (np.array([p[i] for p in products]) for i in range(3))
    want = np.zeros((m * k, k * n, m * n), int)
    for i in range(m):
        for j in range(k):
            for l in range(n):
                want[i * k + j, j * n + l, i * n + l] = 1
    assert (np.einsum("ra,rb,rc->abc", U, V, W) == want).all()
    return shape, U, V, W


SCHEME1 = _scheme((2, 3, 3), [
    ([0, 0, 0, 0, 0, -1], [0, 0, 0, -1, 0, 0, -1, 1, 0], [-1, 0, 0, 1, 0, 0]),
    ([-1, -1, 0, -1, -1, 0], [0, 0, 1, 1, 0, 0, 0, 0, 0], [0, 0, 0, 0, 0, -1]),
    ([1, 0, 1, 0, 0, 0], [0, 0, 0, 0, 0, 0, 0, -1, 0], [-1, -1, 0, 1, 1, 0]),
    ([1, 0, 0, 0, 0, 0], [0, 1, -1, 0, -1, 1, 0, -1, 0], [0, 1, 0, 0, 0, 0]),
    ([0, 0, 0, 0, 1, 0], [0, 0, 0, 0, -1, 0, 0, 0, 0], [0, 1, 1, 0, -1, -1]),
    ([-1, -1, 0, 0, 0, -1], [0, 0, 0, -1, 0, 0, 0, 0, 1], [1, 0, 0, 0, 0, -1]),
    ([1, 1, 0, 0, 1, 0], [0, 0, -1, 0, -1, 1, 0, 0, 0], [0, -1, -1, 0, 0, 1]),
    ([0, 0, 0, -1, 0, 0], [-1, 1, 0, 1, 0, 0, 0, 0, 0], [0, 0, 0, 0, -1, 0]),
    ([0, 0, -1, 0, 0, -1], [-1, 0, 0, 1, 0, 0, 1, 0, 1], [-1, 0, 0, 0, 0, 0]),
    ([0, 1, 0, 0, 1, 0], [0, 0, 1, 0, 0, -1, 0, 0, 0], [0, -1, -1, 0, 0, 0]),
    ([-1, 0, -1, 0, 0, -1], [1, 0, 0, -1, 0, 0, 0, -1, 0], [-1, 0, 0, 1, 1, 0]),
    ([-1, -1, 1, 0, 0, 0], [0, 0, 0, 0, 0, 0, 0, 0, -1], [1, 0, -1, 0, 0, 0]),
    ([-1, 0, -1, -1, 0, -1], [-1, 0, 0, 1, 0, 0, 0, 0, 0], [0, 0, 0, 1, 1, 0]),
    ([0, 0, 0, 1, 1, -1], [0, 0, 0, 1, 0, 0, 0, 0, 0], [0, 0, 0, 1, 0, -1]),
    ([-1, -1, 0, 0, 0, 0], [0, 0, 0, 0, -1, 1, 0, 0, 1], [0, 0, -1, 0, 0, 1]),
])
SCHEME2 = _scheme((2, 3, 3), [
    ([0, 0, 0, 0, 0, 1], [1, 0, 1, 0, 0, 0, -1, 0, 0], [-1, 0, 0, -1, 0, 0]),
    ([1, 0, 0, -1, 1, 0], [0, 0, -1, 0, -1, 0, 0, 0, 0], [1, -1, -1, 0, -1, 0]),
    ([0, -1, -1, 0, 0, 1], [0, 0, 0, -1, 0, -1, 0, 0, 1], [1, 0, 0, 0, 0, 1]),
    ([1, 0, 1, 0, 0, 0], [0, 0, 0, 0, 0, 0, 0, -1, 0], [-1, -1, 0, 0, 0, 0]),
    ([0, 0, 0, -1, 0, -1], [-1, 0, -1, 0, 0, 0, 0, 0, 0], [0, 0, 0, 1, 1, 0]),
    ([-1, 0, 0, 0, 0, -1], [1, 0, 1, 0, 0, 0, 0, -1, 0], [-1, 0, 0, 0, 1, 0]),
    ([0, 1, 0, 0, 0, 0], [0, 0, 0, 0, -1, 1, 0, 0, -1], [-1, 0, 1, 0, 0, 0]),
    ([0, 0, 1, 0, 0, -1], [0, 0, 0, -1, 0, -1, 1, -1, 1], [1, 0, 0, 0, 0, 0]),
    ([-1, 0, 0, 0, 0, 0], [0, 1, -1, 0, 0, 0, 0, -1, 0], [0, -1, 0, 0, -1, 0]),
    ([0, -1, -1, 0, 1, 1], [0, 0, 0, 1, 0, 1, 0, 0, 0], [0, 0, 0, 0, 0, 1]),
    ([0, 0, 0, 0, 1, 0], [0, 0, -1, 1, 0, 0, 0, 0, 0], [0, 0, 0, 1, 0, -1]),
    ([-1, 1, 0, 1, -1, 0], [0, 0, 0, 0, 1, 0, 0, 0, 0], [-1, 1, 1, 0, 0, 0]),
    ([0, 0, 0, 1, -1, 0], [0, 0, 1, 0, 0, 0, 0, 0, 0], [-1, 1, 1, -1, 1, 1]),
    ([0, -1, -1, 0, 0, 0], [0, 0, 0, 0, 0, 0, 0, 0, -1], [0, 0, 1, 0, 0, 1]),
    ([1, 0, 0, -1, 0, 0], [-1, 1, -1, 0, 1, 0, 0, 0, 0], [0, 0, 0, 0, -1, 0]),
])


def cse(rows):
    R = [list(map(int, r)) for r in rows]; steps = []
    while True:
        n = len(R[0]); best = 1; arg = None
        for i in range(n):
            for j in range(i+1, n):
                a = sum(1 for r in R if r[i]*r[j] > 0); b = sum(1 for r in R if r[i]*r[j] < 0)
                if a > best: best = a; arg = (i, j, 1)
                if b > best: best = b; arg = (i, j, -1)
        if arg is None: break
        i, j, s = arg; steps.append(arg)
        for r in R:
            if r[i]*r[j] == s: r.append(r[i]); r[i] = 0; r[j] = 0
            else: r.append(0)
    return steps, [[(v, c) for v, c in enumerate(r) if c] for r in R]


def lincomb(terms, get):
    pos = [v for v, c in terms if c > 0]
    neg = [v for v, c in terms if c < 0]
    sign = 1
    if not pos:
        pos, neg, sign = neg, [], -1
    acc = get(pos[0])
    for v, c in terms:
        if v == pos[0]:
            continue
        acc = acc + get(v) if c * sign > 0 else acc - get(v)
    return acc, sign


class Lazy:
    def __init__(self, nin, steps, leaf):
        self.nin, self.steps, self.leaf, self.memo = nin, steps, leaf, {}
    def __call__(self, v):
        if v not in self.memo:
            if v < self.nin:
                self.memo[v] = self.leaf(v)
            else:
                i, j, s = self.steps[v - self.nin]
                self.memo[v] = self(i) + self(j) if s > 0 else self(i) - self(j)
        return self.memo[v]


def schedule(T, S, NS, D):
    spread = S - NS
    keep = [((i + 1) * spread) // (T - NS) > (i * spread) // (T - NS) for i in range(T - NS)] + [True] * NS
    slot1, spill, wait1, last, nxt, rr, nsp = [], [], [], {}, NS, 0, 0
    for i in range(T):
        if keep[i] and i < T - NS:
            slot1.append(nxt); wait1.append(-1); nxt += 1
        else:
            slot1.append(rr); wait1.append(last.get(rr, -1)); last[rr] = i; rr = (rr + 1) % NS
        spill.append(-1 if keep[i] else nsp)
        nsp += not keep[i]
    kept = [i for i in range(T) if keep[i]][::-1]
    rest = [i for i in range(T) if not keep[i]]
    order, nk = kept[:D], len(kept) - D
    kept = kept[D:]
    for j in range(T - D):
        order.append(kept.pop(0) if ((j + 1) * nk) // (T - D) > (j * nk) // (T - D) else rest.pop(0))
    slot2 = []
    for j, i in enumerate(order):
        slot2.append(slot1[i] if keep[i] else slot2[j - D])
    src2 = [spill[i] for i in order]
    wsp = [spill[w] if w >= 0 else -1 for w in wait1]
    return np.array([slot1, spill, wsp, order, slot2, src2], np.int32), nsp


def fold_triangles(W):
    R = len(W)
    tri = [(p, q, r, a, b) for p in range(R) for q in range(p + 1, R) for r in range(R) for a in (1, -1) for b in (1, -1)
           if r != p and r != q and (W[r] == a * W[p] + b * W[q]).all()]
    def cost(sel):
        keep = [i for i in range(R) if i not in [t[2] for t in sel]]
        steps, outs = cse(W[keep].T)
        return 2 * len(sel) + len(steps) + sum(len(t) - 1 for t in outs)
    level, best = [()], ()
    while level:
        best = min(level, key=cost)
        level = [sel + (t,) for sel in level for t in tri
                 if (not sel or t > sel[-1]) and not set(t[:3]) & set(i for u in sel for i in u[:3])]
    return best


RB1 = 128
U1 = 4
TP = 2
RB2 = 128
U2 = 4
NX = 5
XA = 3
S = 37
NS = 5
D = 3
ST = 16
lag1 = 6
gd = 2
lnhi = 0.85
lnlag = 4
nln = 4
pmode = 8
mdel = 2
pdel = 3
LN = 8
ST2 = 32
lag2 = 1
cbhi = 0.9
cd = 1


@jax.jit
def pallas_standalone__modern_conv_block_slak__vision_kernel(x, dw, w1, w2, grn_g, grn_b):
    B, H, W, C = x.shape
    assert B == 1 and dw.shape[:2] == (1, 1)
    F = w1.shape[1]
    N = B * H * W
    f32, bf16, u32 = jnp.float32, jnp.bfloat16, jnp.uint32
    (m1, k1, n1), Us1, Vs1, Ws1 = SCHEME1
    (m2, k2, n2), Us2, Vs2, Ws2 = SCHEME2
    R1, R2 = len(Us1), len(Us2)
    assert k1 * L == C and n2 * L == C
    G1, G2 = F // (n1 * L), F // (k2 * L)
    a1_steps, a1_out = cse(Us1)
    tris = fold_triangles(Ws1)
    kept1 = [r for r in range(R1) if r not in [t[2] for t in tris]]
    K1 = len(kept1)
    c1_steps, c1_out = cse(Ws1[kept1].T)
    loose = [r for r in range(R1) if r not in [i for t in tris for i in t[:3]]]
    UU = U1 * TP
    dots1, pend = [], [(list(tris), [(a, r) for r in loose]) for a in range(UU * G1)]
    for a in range(UU * G1):
        todo, free = pend[a]
        while todo or free:
            if todo and len(dots1) % NM <= 1 and (len(dots1) % NM == 1 or len(free) <= len(todo) or len(tris) < 4):
                dots1 += [(a, r) for r in todo.pop(0)[:3]]
            else:
                dots1.append((free or pend[a + 1][1]).pop(0))
    a2_steps, a2_out = cse(Us2)
    c2_steps, c2_out = cse(Ws2.T)
    sg1 = [1 if any(c > 0 for _, c in t) else -1 for t in a1_out]
    sg2 = [1 if any(c > 0 for _, c in t) else -1 for t in a2_out]
    direct2 = [len(t) == 1 and t[0][0] < m2 * k2 for t in a2_out]
    CM1, CM2 = m1 * RB1, m2 * RB2
    TM = CM1 * U1
    assert TM == CM2 * U2 and N % TM == 0 and U1 % 2 == 0 and U2 % 2 == 0 and (U1 * G1) % 4 == 0
    assert CM2 % RB1 == 0
    T, NT = N // TM, F // L
    tab, nsp = schedule(T, S, NS, D)
    assert T % TP == 0 and NS >= 2 * TP + 1
    M1R, A1R, M2R, A2R = RB1 + 8, RB1 + 16, RB2 + 8, RB2
    HS = NT * TM
    hrow = lambda ct, r: (r // CM2) * (NT * CM2) + ct * CM2 + r % CM2
    MR = max(K1 * M1R, R2 * M2R)
    AR = max(R1 * A1R, R2 * G2 * A2R)
    LR = nln * m1 * 16
    as_u, as_b = (lambda v: pltpu.bitcast(v, u32)), (lambda v: pltpu.bitcast(v, bf16))

    def kernel(tab_ref, x_hbm, dw_ref, w1_hbm, w2_hbm, g_ref, b_ref, o_hbm, h_hbm,
               xbuf, hbuf, wbuf, acc, row, zero, lnbuf, ab0, ab1, mb0, mb1, mb2, mb3, xsem, hsem, osem, wsem):
        abs_, mbs = (ab0, ab1), (mb0, mb1, mb2, mb3)

        mk = pltpu.make_async_copy
        def x_copy(i, s): return mk(x_hbm.at[pl.ds(i * TM, TM)], xbuf.at[s, pl.ds(0, TM)], xsem.at[s])
        def hw_copy(i, s): return mk(hbuf.at[s, pl.ds(0, HS)], h_hbm.at[i], hsem.at[s])
        def hr_head(i, s): return mk(h_hbm.at[i, pl.ds(0, NT * CM2)], hbuf.at[s, pl.ds(0, NT * CM2)], hsem.at[s])
        def hr_rest(i, s): return mk(h_hbm.at[i, pl.ds(NT * CM2, HS - NT * CM2)], hbuf.at[s, pl.ds(NT * CM2, HS - NT * CM2)], hsem.at[S + s])
        def o_copy(i, s): return mk(xbuf.at[s, pl.ds(0, TM)], o_hbm.at[pl.ds(i * TM, TM)], osem.at[s])

        XO = (XA - (T - NX)) % NX
        xslot = lambda i: lax.rem(i + XO, NX)
        ws1, ws2 = [(NX - 2 + c + XO) % NX for c in range(2)], [XA, XA + 1]
        w1_copies = [pltpu.make_async_copy(w1_hbm.at[:, pl.ds(c * C, C)], xbuf.at[ws1[c // 2], pl.ds((c % 2) * C, C)], wsem.at[c])
                     for c in range(4)]
        w2_copies = [pltpu.make_async_copy(w2_hbm.at[pl.ds(c * 2 * C, 2 * C)], xbuf.at[ws2[c], pl.ds(0, 2 * C)], wsem.at[4 + c])
                     for c in range(2)]
        def w1_tile(kt, ct):
            c, j = divmod(ct, C // L)
            return xbuf[ws1[c // 2], (c % 2) * C + kt * L:(c % 2) * C + (kt + 1) * L, j * L:(j + 1) * L].astype(f32)
        def w2_tile(ct, j):
            c, r0 = divmod(ct * L, 2 * C)
            return xbuf[ws2[c], r0:r0 + L, j * L:(j + 1) * L].astype(f32)

        for cp in w1_copies:
            cp.start()
        for j in range(NX - 2):
            x_copy(j, (j + XO) % NX).start()
        zero[0] = 0
        acc[...] = jnp.zeros_like(acc)
        for buf in mbs:
            buf[MR:MR + 24, :] = jnp.zeros((24, L), f32)
        for buf in abs_:
            buf[AR:AR + 16, :] = jnp.zeros((16, L), bf16)
        row[0] = jnp.broadcast_to(dw_ref[...].astype(f32), (8, C))

        def ln_store(s, r0, lrow):
            o = xbuf[s, pl.ds(r0, LN), :].astype(f32) * jnp.concatenate([row[0]] * (LN // 8), axis=0)
            mu = jnp.sum(o, axis=-1, keepdims=True) * (1.0 / C)
            d = o - mu
            v = jnp.sum(d * d, axis=-1, keepdims=True)
            a = d * (lax.rsqrt(v + C * 1e-5) * (_A * C ** 0.5))
            for j in range(k1):
                lnbuf[j, pl.ds(lrow, LN), :] = a[:, j * L:(j + 1) * L]

        def ac_tile(lrow, dst, drow):
            av = Lazy(m1 * k1, a1_steps, lambda v: lnbuf[v % k1, pl.ds(lrow + (v // k1) * 16, 16), :])
            for r in range(R1):
                dst[pl.ds(drow + r * A1R, 16), :] = lincomb(a1_out[r], av)[0].astype(bf16)

        def gelu_rows(getm, g, sq):
            mv = Lazy(K1, c1_steps, getm)
            res = []
            for e in range(m1 * n1):
                y, sg = lincomb(c1_out[e], mv)
                th = jnp.tanh(y * (y * y + _K0))
                hv = y * (th + 1.0) if sg > 0 else y * (th - 1.0)
                ct = (e % n1) * G1 + g
                sq[ct] = sq[ct] + hv * hv if ct in sq else hv * hv
                res.append(hv)
            return res

        def h_store(lo, hi, s, r0, g, dyn=0):
            for e in range(m1 * n1):
                hbuf[s, pl.ds(dyn + hrow((e % n1) * G1 + g, r0 + (e // n1) * RB1), 16), :] = (
                    jnp.concatenate([lo[e], hi[e]], axis=0).astype(bf16))

        def flush_sq(sq):
            for ct in sorted(sq):
                acc[ct] += sq[ct]
            sq.clear()

        tpr = RB1 // ST
        ntick = len(dots1) // NM * tpr
        nt = RB1 // 8
        ge_at = [[] for _ in range(ntick)]
        for a in range(UU * G1):
            ready = (max(z for z, d in enumerate(dots1) if d[0] == a) // NM + 1) * tpr
            for t in range(nt):
                z = max(((a + 1) * R1 * tpr) // NM + lag1 + (t * R1 * tpr) // (NM * nt), ready)
                if t % 2 and z >= ntick > zprev:
                    z = ntick - 1
                zprev = z
                ge_at[z % ntick].append((a, t, z >= ntick))
        carried = sorted({(a, t) for ev in ge_at for a, t, c in ev if c})
        per16 = m1 * (16 // LN)
        ln_at, ac_at = [[] for _ in range(ntick)], [[] for _ in range(ntick)]
        for u in range(UU):
            n_it = RB1 // 16 * per16
            for it in range(n_it):
                z = int((u + lnhi * it / n_it) * ntick / UU)
                ln_at[z].append((u + 1, it // per16, it % per16))
                if (it + 1) % per16 == 0:
                    ac_at[z + lnlag].append((u + 1, it // per16))

        def p1_body(hs, xs, par):
            zp = pl.multiple_of(8 * par, 8)
            z0 = pl.multiple_of(zero[0], 16)
            sq, held, done, probes = {}, [], [], []
            for rho in range(len(dots1) // NM):
                res = []
                for a, r in dots1[rho * NM:(rho + 1) * NM]:
                    lhs = abs_[(a // G1) % 2][r * A1R:r * A1R + RB1, :]
                    res.append((a, r, jnp.dot(lhs, as_b(wbuf[(a % G1) * R1 + r]), preferred_element_type=f32)))
                for k in range(tpr):
                    pv = res[0][2][k * ST:k * ST + 8]
                    got = {(a, r): val[k * ST:(k + 1) * ST] for a, r, val in res}
                    for p, q, r, ca, cb in tris:
                        for a in sorted({a for a, r2 in got if r2 == r}):
                            m = got.pop((a, r))
                            got[a, p] = got[a, p] + m if ca > 0 else got[a, p] - m
                            got[a, q] = got[a, q] + m if cb > 0 else got[a, q] - m
                    for (a, r), val in got.items():
                        mbs[a % 4][pl.ds(z0 + kept1.index(r) * M1R + k * ST, ST), :] = val
                    if k % pmode == pmode - 1:
                        for a in sorted({a for a, _, _ in res}):
                            probes.append((len(done) + mdel, mbs[a % 4][MR + 16:MR + 24, :]))
                        probes.sort(key=lambda e: e[0])
                    for (pa, t, c) in ge_at[rho * tpr + k]:
                        pu, pg = divmod(pa, G1)
                        val = pv
                        if len(done) >= gd:
                            val = done[-gd] + pv
                            while probes and probes[0][0] <= len(done):
                                val = val + probes.pop(0)[1]
                        mbs[pa % 4][pl.ds(MR + zp, 8), :] = val
                        held.append(gelu_rows(lambda v: mbs[pa % 4][v * M1R + t * 8:v * M1R + (t + 1) * 8, :], pg, sq))
                        done.append(sum([sq[l * G1 + pg] for l in range(1, n1)], sq[pg]))
                        if len(held) == 2:
                            h_store(held[0], held[1], hs[0 if c else 1 + pu // U1], (pu % U1) * CM1 + (t - 1) * 8, pg)
                            held = []
                        if t == nt - 1:
                            flush_sq(sq)
                    for (nu, t, j) in ln_at[rho * tpr + k]:
                        q, j2 = divmod(j, 16 // LN)
                        ln_store(xs[nu // U1], (nu % U1) * CM1 + q * RB1 + t * 16 + j2 * LN,
                                 z0 + (t % nln) * m1 * 16 + j * LN)
                    for (nu, t) in ac_at[rho * tpr + k]:
                        lnbuf[0, pl.ds(LR + zp, 8), :] = pv
                        ac_tile((t % nln) * m1 * 16, abs_[nu % 2], z0 + t * 16)
                        probes.append((len(done) + pdel, abs_[nu % 2][AR:AR + 8, :].astype(f32)))
            flush_sq(sq)

        for a in sorted({a % 4 for a, _ in carried}):
            mbs[a][0:K1 * M1R, :] = jnp.zeros((K1 * M1R, L), f32)
        for cp in w1_copies:
            cp.wait()
        for g in range(G1):
            for r in range(R1):
                val, sg = lincomb([(v, int(c) * sg1[r]) for v, c in enumerate(Vs1[r]) if c],
                                  lambda v: w1_tile(v // n1, (v % n1) * G1 + g))
                wbuf[g * R1 + r] = as_u((val if sg > 0 else -val).astype(bf16))

        for j in range(NX - 2, NX):
            x_copy(j, (j + XO) % NX).start()
        x_copy(0, XO).wait()

        def pro(t, _):
            for j in range(per16):
                q, j2 = divmod(j, 16 // LN)
                ln_store(XO, pl.multiple_of(t * 16, 16) + q * RB1 + j2 * LN, j * LN)
            ac_tile(0, ab0, pl.multiple_of(t * 16, 16))
        lax.fori_loop(0, RB1 // 16, pro, None)

        def p1(it, _):
            i = it * TP
            for d in range(TP):
                @pl.when(i + d + 1 < T)
                def _():
                    x_copy(i + d + 1, xslot(i + d + 1)).wait()

                @pl.when(tab_ref[2, i + d] >= 0)
                def _():
                    hw_copy(tab_ref[2, i + d], tab_ref[0, i + d]).wait()
            p1_body([jnp.where(i > 0, tab_ref[0, jnp.maximum(i - 1, 0)], S - 1)] + [tab_ref[0, i + d] for d in range(TP)],
                    [xslot(jnp.minimum(i + d, T - 1)) for d in range(TP + 1)], lax.rem(it, 2))
            for d in range(TP):
                @pl.when(i + d + NX < T)
                def _():
                    x_copy(i + d + NX, xslot(i + d)).start()

            @pl.when(it == (T - NX + 1) // TP)
            def _():
                for cp in w2_copies:
                    cp.start()
            for d in range(TP):
                ip = jnp.maximum(i + d - 1, 0)

                @pl.when(jnp.logical_and(i + d >= 1, tab_ref[1, ip] >= 0))
                def _():
                    hw_copy(tab_ref[1, ip], tab_ref[0, ip]).start()
        lax.fori_loop(0, T // TP, p1, None)
        for j in range(XA):
            x_copy(int(tab[3, j]), j).start()
        for a in sorted({a for a, _ in carried}):
            def epi(t, _):
                sq = {}
                r0 = pl.multiple_of(t * 16, 16)
                lo, hi = (gelu_rows(lambda v: mbs[a % 4][pl.ds(v * M1R + r0 + 8 * i, 8), :], a % G1, sq) for i in range(2))
                h_store(lo, hi, int(tab[0, T - 1]), ((a // G1) % U1) * CM1, a % G1, r0)
                flush_sq(sq)
            lax.fori_loop(min(t for ca, t in carried if ca == a) // 2, nt // 2, epi, None)
        for cp in w2_copies:
            cp.wait()

        ss = jnp.concatenate([jnp.sum(acc[c], axis=0, keepdims=True) for c in range(NT)], axis=1) * (_GS * _GS)
        gx = jnp.sqrt(ss + 1e-6)
        nx = gx / (jnp.sum(gx, axis=-1, keepdims=True) * (1.0 / F) + 1e-6)
        sc = (g_ref[...].astype(f32).reshape(1, F) * nx + 1.0) * _GS
        sct = jnp.transpose(jnp.broadcast_to(sc, (L, F)))
        bt = jnp.transpose(jnp.broadcast_to(b_ref[...].astype(f32).reshape(1, F), (L, F)))
        for q in range(G2):
            for r in range(R2):
                def get(v):
                    ct = (v // n2) * G2 + q
                    return w2_tile(ct, v % n2) * sct[ct * L:(ct + 1) * L]
                val, sg = lincomb([(v, int(c) * sg2[r]) for v, c in enumerate(Vs2[r]) if c], get)
                wbuf[r * G2 + q] = as_u((val if sg > 0 else -val).astype(bf16))
        for j in range(n2):
            p = sum(w2_tile(ct, j) * bt[ct * L:(ct + 1) * L] for ct in range(NT))
            row[1, :, j * L:(j + 1) * L] = jnp.broadcast_to(jnp.sum(p, axis=0, keepdims=True), (8, L))
        mb1[0:R2 * M2R, :] = jnp.zeros((R2 * M2R, L), f32)

        def comb_tile(s, r0, q, dst, drow, dyn=0):
            raw = Lazy(m2 * k2, [], lambda v: hbuf[s, pl.ds(dyn + hrow((v % k2) * G2 + q, r0 + (v // k2) * RB2), 16), :])
            av = Lazy(m2 * k2, a2_steps, lambda v: raw(v).astype(f32))
            for r in range(R2):
                dst[pl.ds(drow + (r * G2 + q) * A2R, 16), :] = (
                    raw(a2_out[r][0][0]) if direct2[r] else lincomb(a2_out[r], av)[0].astype(bf16))

        def out_tile(src, srow, sx, r0):
            mv = Lazy(R2, c2_steps, lambda v: src[pl.ds(srow + v * M2R, 16), :])
            for i in range(m2):
                rows = pl.ds(r0 + i * RB2, 16)
                xv = xbuf[sx, rows, :].astype(f32) + jnp.concatenate([row[1]] * 2, axis=0)
                res = []
                for l in range(n2):
                    y, sg = lincomb(c2_out[i * n2 + l], mv)
                    z = xv[:, l * L:(l + 1) * L]
                    res.append(z + y if sg > 0 else z - y)
                xbuf[sx, rows, :] = jnp.concatenate(res, axis=1).astype(bf16)

        tp2 = RB2 // ST2
        ntick2 = U2 * R2 * tp2
        nt2 = RB2 // 16
        ot_at, cb_at = [[] for _ in range(ntick2)], [[] for _ in range(ntick2)]
        for u in range(U2):
            for t in range(nt2):
                z = (u + 1) * R2 * tp2 + lag2 + (t * (R2 * tp2 - lag2)) // nt2
                ot_at[z % ntick2].append((u, t, z >= ntick2))
            for k in range(G2 * nt2):
                cb_at[int((u + cbhi * k / (G2 * nt2)) * R2 * tp2)].append((u + 1, k % G2, k // G2))

        def p2_body(sx_prev, sx_cur, s_cur, s_next, par):
            z0 = pl.multiple_of(zero[0], 16)
            probes, ncb = [], 0
            for z in range(U2 * R2):
                u, r = divmod(z, R2)
                ys = [jnp.dot(abs_[u % 2][(r * G2 + q) * A2R:(r * G2 + q) * A2R + RB2, :], as_b(wbuf[r * G2 + q]),
                              preferred_element_type=f32) for q in range(G2)]
                val = (ys[0] + ys[1]) + (ys[2] + ys[3])
                for k in range(tp2):
                    pv = val[k * ST2:k * ST2 + 8]
                    mbs[u % 2][pl.ds(z0 + r * M2R + k * ST2, ST2), :] = val[k * ST2:(k + 1) * ST2]
                    for (pu, t, c) in ot_at[z * tp2 + k]:
                        mbs[pu % 2][pl.ds(MR + pl.multiple_of(8 * par, 8), 8), :] = pv
                        xbuf[z0, TM:TM + 8, 0:L] = pv.astype(bf16)
                        out_tile(mbs[pu % 2], t * 16, sx_prev if c else sx_cur, pu * CM2 + t * 16)
                    for (nu, q, t) in cb_at[z * tp2 + k]:
                        pin = pv
                        while probes and probes[0][0] <= ncb:
                            pin = pin + probes.pop(0)[1]
                        hbuf[z0, HS:HS + 8, :] = pin.astype(bf16)
                        comb_tile(s_cur if nu < U2 else s_next, (nu % U2) * CM2 + t * 16, q, abs_[nu % 2], z0 + t * 16)
                        ncb += 1
                        probes.append((ncb + cd, abs_[nu % 2][AR:AR + 8, :].astype(f32)))

        def pro2(t, _):
            r0 = pl.multiple_of(t * 16, 16)
            for q in range(G2):
                comb_tile(int(tab[4, 0]), 0, q, ab0, r0, r0)
        lax.fori_loop(0, nt2, pro2, None)

        def p2(j, _):
            jn, jd, jp = jnp.minimum(j + 1, T - 1), jnp.minimum(j + D, T - 1), jnp.maximum(j - 1, 0)

            @pl.when(jnp.logical_and(j + 1 < T, tab_ref[5, jn] >= 0))
            def _():
                hr_head(tab_ref[5, jn], tab_ref[4, jn]).wait()

            @pl.when(tab_ref[5, j] >= 0)
            def _():
                hr_rest(tab_ref[5, j], tab_ref[4, j]).wait()
            x_copy(tab_ref[3, j], lax.rem(j, NX)).wait()
            p2_body(lax.rem(j + NX - 1, NX), lax.rem(j, NX), tab_ref[4, j], tab_ref[4, jn], lax.rem(j, 2))

            @pl.when(j >= 1)
            def _():
                o_copy(tab_ref[3, jp], lax.rem(jp, NX)).start()

            @pl.when(j + XA >= NX)
            def _():
                o_copy(tab_ref[3, jnp.maximum(j + XA - NX, 0)], lax.rem(j + XA, NX)).wait()

            @pl.when(j + XA < T)
            def _():
                x_copy(tab_ref[3, jnp.minimum(j + XA, T - 1)], lax.rem(j + XA, NX)).start()

            @pl.when(jnp.logical_and(j + D < T, tab_ref[5, jd] >= 0))
            def _():
                hr_head(tab_ref[5, jd], tab_ref[4, jd]).start()
                hr_rest(tab_ref[5, jd], tab_ref[4, jd]).start()
        lax.fori_loop(0, T, p2, None)

        def epi2(t, _):
            r0 = pl.multiple_of(t * 16, 16)
            out_tile(mb1, r0, (T - 1) % NX, (U2 - 1) * CM2 + r0)
        lax.fori_loop(0, nt2, epi2, None)
        o_copy(int(tab[3, T - 1]), (T - 1) % NX).start()
        for j in range(T + XA - NX, T):
            o_copy(int(tab[3, j]), j % NX).wait()

    vm = pl.BlockSpec(memory_space=pltpu.VMEM)
    hb = pl.BlockSpec(memory_space=pl.ANY)
    out, _ = pl.pallas_call(
        kernel,
        in_specs=[pl.BlockSpec(memory_space=pltpu.SMEM), hb, vm, hb, hb, vm, vm],
        out_specs=[hb, hb],
        out_shape=[jax.ShapeDtypeStruct((N, C), bf16), jax.ShapeDtypeStruct((nsp, HS, L), bf16)],
        scratch_shapes=[
            pltpu.VMEM((NX, TM + 16, C), bf16), pltpu.VMEM((S, HS + 16, L), bf16),
            pltpu.VMEM((max(G1 * R1, G2 * R2), L // 2, L), u32), pltpu.VMEM((NT, 8, L), f32), pltpu.VMEM((2, 8, C), f32),
            pltpu.SMEM((1,), jnp.int32), pltpu.VMEM((k1, LR + 16, L), f32),
            *[pltpu.VMEM((AR + 16, L), bf16)] * 2, *[pltpu.VMEM((MR + 24, L), f32)] * 4,
            pltpu.SemaphoreType.DMA((NX,)), pltpu.SemaphoreType.DMA((2 * S,)), pltpu.SemaphoreType.DMA((NX,)),
            pltpu.SemaphoreType.DMA((6,)),
        ],
        compiler_params=pltpu.CompilerParams(vmem_limit_bytes=128 * 1024 * 1024, disable_bounds_checks=True),
    )(tab, x.reshape(N, C), dw.reshape(1, C), w1, w2, grn_g, grn_b)
    return out.reshape(B, H, W, C)
```
